```python
import jax
import jax.numpy as jnp

def _softmax(x, axis=-1):
    return jax.nn.softmax(x, axis=axis)

def _gelu(x):
    return jax.nn.gelu(x, approximate=True)

def _silu(x):
    return jax.nn.silu(x)

def _sigmoid(x):
    return jax.nn.sigmoid(x)

def _layernorm(x, axis=-1, eps=1e-05):
    m = jnp.mean(x, axis=axis, keepdims=True)
    v = jnp.var(x, axis=axis, keepdims=True)
    return (x - m) / jnp.sqrt(v + eps)

def _scatter_add(tgt, idx, src, axis=0):
    return tgt.at[idx].add(src)

def _segment_sum(src, seg, n):
    return jax.ops.segment_sum(src, seg, n)

class _Rng:

    def __init__(self, key):
        self._k = key

    def _next(self):
        self._k, sub = jax.random.split(self._k)
        return sub

    def normal(self, shape):
        return jax.random.normal(self._next(), shape, dtype=jnp.bfloat16)

    def randint(self, lo, hi, shape):
        return jax.random.randint(self._next(), shape, lo, hi, dtype=jnp.int32)

    def uniform(self, shape, lo=0.0, hi=1.0):
        return jax.random.uniform(self._next(), shape, jnp.bfloat16, lo, hi)

    def permutation(self, n):
        return jax.random.permutation(self._next(), n)
kernel_name = 'gated_mix__memory_aug_recurrent_mem_tr__sliding_local_dilated__prompt'

def setup_inputs():
    _rng = _Rng(jax.random.key(int.from_bytes(__import__("os").urandom(4), "little")))
    _w = lambda a: (lambda t: t.astype(jnp.bfloat16) if jnp.issubdtype(t.dtype, jnp.floating) else t)(jnp.asarray(a))

    def _A_setup():
        B, S, Dm = (1, 2048, 640)
        H, Dh = (32, 192)
        M, seg = (8, 32)
        seg = min(seg, S)
        S = S // seg * seg
        return {'x': _w((lambda *s: _rng.normal(s) * 0.05)(B, S, Dm)), 'mem0': _w((lambda *s: _rng.normal(s) * 0.05)(B, M, Dm)), 'Wq': _w((lambda *s: _rng.normal(s) * 0.05)(Dm, H, Dh) * Dm ** (-0.5)), 'Wk': _w((lambda *s: _rng.normal(s) * 0.05)(Dm, H, Dh) * Dm ** (-0.5)), 'Wv': _w((lambda *s: _rng.normal(s) * 0.05)(Dm, H, Dh) * Dm ** (-0.5)), 'Wo': _w((lambda *s: _rng.normal(s) * 0.05)(H, Dh, Dm) * (H * Dh) ** (-0.5)), 'seg_len': seg}
    _A_in = _A_setup()

    def _B_setup():
        B, S, D = (1, 2048, 640)
        return {'x': _w((lambda *s: _rng.normal(s) * 0.05)(B, S, D)), 'wqkv': _w((lambda *s: _rng.normal(s) * 0.05)(D, 3 * D)), 'wo': _w((lambda *s: _rng.normal(s) * 0.05)(D, D))}
    _B_in = _B_setup()
    return {'A_x': _A_in['x'], 'A_mem0': _A_in['mem0'], 'A_Wq': _A_in['Wq'], 'A_Wk': _A_in['Wk'], 'A_Wv': _A_in['Wv'], 'A_Wo': _A_in['Wo'], 'A_seg_len': _A_in['seg_len'], 'B_x': _B_in['x'], 'B_wqkv': _B_in['wqkv'], 'B_wo': _B_in['wo'], 'gate_w': _w((lambda *s: _rng.normal(s) * 0.05)(640))}

def reference(A_x, A_mem0, A_Wq, A_Wk, A_Wv, A_Wo, A_seg_len, B_x, B_wqkv, B_wo, gate_w):

    def _A_ref(x, mem0, Wq, Wk, Wv, Wo, seg_len):
        B, S, Dm = x.shape
        H, Dh = (Wq.shape[1], Wq.shape[2])
        M = mem0.shape[1]
        scale = Dh ** (-0.5)
        n_seg = S // seg_len
        L = M + seg_len
        idx = jnp.arange(L)
        mask = (idx[:, None] < M) | (idx[:, None] >= idx[None, :])
        mem = mem0
        outs = []
        for s in range(n_seg):
            xs = x[:, s * seg_len:(s + 1) * seg_len, :].copy()
            h = jnp.concatenate([mem, xs], axis=1)
            q = jnp.einsum('btd,dhe->bhte', h, Wq)
            k = jnp.einsum('btd,dhe->bhte', h, Wk)
            v = jnp.einsum('btd,dhe->bhte', h, Wv)
            scores = jnp.einsum('bhqe,bhke->bhqk', q, k) * scale
            scores = jnp.where(mask[None, None], scores, -1000000000.0)
            p = _softmax(scores, axis=-1)
            o = jnp.einsum('bhqk,bhke->bhqe', p, v)
            o = jnp.einsum('bhte,hed->btd', o, Wo)
            mem = o[:, :M, :].copy()
            outs.append(o[:, M:, :])
        return jnp.concatenate(outs, axis=1)

    def _B_ref(x, wqkv, wo):
        B, S, D = x.shape
        H = 32
        Dh = D // H
        W, dil = (8, 2)
        qkv = (lambda x, *d: x.transpose(*d))((x @ wqkv).reshape(B, S, 3, H, Dh), 2, 0, 3, 1, 4)
        q, k, v = (qkv[0], qkv[1], qkv[2])
        scale = Dh ** (-0.5)
        pos = jnp.arange(S)
        off = jnp.arange(W) * dil
        idx = pos[:, None] - off[None, :]
        mask = idx >= 0
        idx_c = jnp.where(mask, idx, 0).reshape(-1)
        kg = k[:, :, idx_c, :].reshape(B, H, S, W, Dh)
        vg = v[:, :, idx_c, :].reshape(B, H, S, W, Dh)
        logits = jnp.einsum('bhsd,bhswd->bhsw', q, kg) * scale
        logits = jnp.where(mask[None, None, :, :], logits, -1000000000.0)
        attn = _softmax(logits, axis=-1)
        o = jnp.einsum('bhsw,bhswd->bhsd', attn, vg)
        return (lambda x, *d: x.transpose(*d))(o, 0, 2, 1, 3).reshape(B, S, D) @ wo
    x = A_x
    g = _sigmoid((x * gate_w).sum(-1, keepdims=True))
    a = _A_ref(x, A_mem0, A_Wq, A_Wk, A_Wv, A_Wo, A_seg_len)
    b = _B_ref(x, B_wqkv, B_wo)
    return g * a + (1 - g) * b
```

```python
import functools

import jax
import jax.numpy as jnp
from jax.experimental import pallas as pl
from jax.experimental.pallas import tpu as pltpu

F32 = jnp.float32
BF16 = jnp.bfloat16
U32 = jnp.uint32

S = 2048
D = 640
H = 32
DH = 192
M = 8
SEG = 32
L = M + SEG
NSEG = S // SEG
NP = H // 2
PW = 2 * DH
MASK_VALUE = -1e9
LOG2E = 1.4426950408889634
HB = 32
DB = D // HB
WIN = 8
DIL = 2
RB = 64
NB = S // RB
HALO = 16
NT_ = D // 128

NSLOT = 6
AHEAD = 4

NN = (((1,), (0,)), ((), ()))
NT = (((1,), (1,)), ((), ()))


def _dot(a, b, dims=NN):
    return jax.lax.dot_general(a, b, dims, preferred_element_type=F32)


def _w(x):
    return pltpu.bitcast(x, BF16)


def _pack(x):
    return pltpu.bitcast(x, U32)


def _recip(den):
    r = pl.reciprocal(den, approx=True)
    return r * (2.0 - den * r)


def _blockdiag(t):
    lo = jax.lax.broadcasted_iota(jnp.int32, (L, 128), 1) < 64
    z = jnp.zeros((L, 128), F32)
    t0, t1, t2 = t[:, 0:128], t[:, 128:256], t[:, 256:384]
    top = jnp.concatenate([t0, jnp.where(lo, t1, 0.0), z], axis=1)
    bot = jnp.concatenate([z, jnp.where(lo, 0.0, t1), t2], axis=1)
    return jnp.concatenate([top, bot], axis=0).astype(BF16)


def _kernel(xa_hbm, mem_ref, wq_hbm, wk_hbm, wv_hbm, wo_hbm,
            wqkvb_hbm, wob_hbm, gate_ref,
            out_hbm,
            xa_v, out_v, b_v, h_ref,
            stage, w32, wo32,
            wqkvb_v, wob_v, wqkvb32, wob32, prep, slab0, slab1, obuf0, obuf1,
            sem_w, sem_in, sem_out):
    def pair_copies(p, slot):
        rows = pl.ds(pl.multiple_of(p * PW, 128), PW)
        return [pltpu.make_async_copy(src.at[rows, :], stage.at[slot, i], sem_w.at[p])
                for i, src in enumerate((wq_hbm, wk_hbm, wv_hbm, wo_hbm))]

    c_wqkvb = pltpu.make_async_copy(wqkvb_hbm, wqkvb_v, sem_in.at[0])
    c_wob = pltpu.make_async_copy(wob_hbm, wob_v, sem_in.at[1])
    c_xa = pltpu.make_async_copy(xa_hbm, xa_v, sem_in.at[2])
    c_wqkvb.start()
    c_wob.start()
    c_xa.start()
    for p in range(AHEAD):
        for c in pair_copies(p, p):
            c.start()

    c_wqkvb.wait()
    for c in range(3 * NT_):
        t = wqkvb_v[:, c * 128:(c + 1) * 128].astype(F32).T
        for kt in range(NT_):
            prep[kt, c * 128:(c + 1) * 128, :] = t[:, kt * 128:(kt + 1) * 128]
    for part in range(3):
        for d in range(DB):
            rows = jnp.concatenate(
                [prep[kt, pl.ds(part * D + d, HB, stride=DB), :] for kt in range(NT_)], axis=1)
            r0 = (part * D + d * HB) // 2
            wqkvb32[r0:r0 + HB // 2, :] = _pack(rows.astype(BF16))
    c_wob.wait()
    for kt in range(NT_):
        prep[kt, 0:D, :] = wob_v[:, kt * 128:(kt + 1) * 128].astype(F32)
    for d in range(DB):
        rows = jnp.concatenate(
            [prep[kt, pl.ds(d, HB, stride=DB), :] for kt in range(NT_)], axis=1)
        wob32[d * (HB // 2):(d + 1) * (HB // 2), :] = _pack(rows.astype(BF16))

    def b_project(blk, dst, prev):
        x = xa_v[pl.ds(pl.multiple_of(blk * RB, RB), RB), :]
        for j in range(3 * NT_):
            dst[j, HALO:HALO + RB, :] = _dot(x, _w(wqkvb32[j * 64:(j + 1) * 64, :]), NT)
        for j in range(NT_, 3 * NT_):
            if prev is None:
                dst[j, 0:HALO, :] = jnp.zeros((HALO, 128), F32)
            else:
                dst[j, 0:HALO, :] = prev[j, RB:RB + HALO, :]

    def b_attend_rows(src, base, n, row0):
        q = [src[j, HALO + base:HALO + base + n, :] for j in range(NT_)]
        row = jax.lax.broadcasted_iota(jnp.int32, (n, 128), 0) + (row0 + base)
        logits = []
        for w in range(WIN):
            o = HALO + base - DIL * w
            s = q[0] * src[NT_, o:o + n, :]
            for j in range(1, NT_):
                s = s + q[j] * src[NT_ + j, o:o + n, :]
            s = s + pltpu.roll(s, 64, 1)
            s = s + pltpu.roll(s, 32, 1)
            s = s * (DB ** -0.5 * LOG2E)
            if w:
                s = jnp.where(row >= DIL * w, s, MASK_VALUE * LOG2E)
            logits.append(s)
        m = logits[0]
        for w in range(1, WIN):
            m = jnp.maximum(m, logits[w])
        e = [jnp.exp2(l - m) for l in logits]
        den = e[0]
        for w in range(1, WIN):
            den = den + e[w]
        r = _recip(den)
        outs = []
        for j in range(NT_):
            acc = None
            for w in range(WIN):
                o = HALO + base - DIL * w
                t = e[w] * src[2 * NT_ + j, o:o + n, :]
                acc = t if acc is None else acc + t
            outs.append(acc * r)
        return jnp.concatenate(outs, axis=1)

    def b_attend(blk, src, o_dst):
        o_dst[...] = b_attend_rows(src, 0, RB, blk * RB)

    def b_output(blk, o_src):
        b_v[pl.ds(pl.multiple_of(blk * RB, RB), RB), :] = _dot(o_src[...], _w(wob32[...]))

    def a_weights(p, slot):
        col = pl.multiple_of(p * 3 * PW, 128)
        for i in range(3):
            w32[:, pl.ds(col + i * PW, PW)] = _pack(stage[slot, i].astype(F32).T.astype(BF16))
        wo32[pl.ds(pl.multiple_of(p * (PW // 2), 64), PW // 2), :] = _pack(stage[slot, 3])

    def start_pair(p):
        for c in pair_copies(p, p % NSLOT):
            c.start()

    def wait_pair(p):
        for c in pair_copies(p, p % NSLOT):
            c.wait()

    c_xa.wait()
    b_project(0, slab0, None)
    start_pair(AHEAD)
    b_project(1, slab1, slab0)
    b_attend(0, slab0, obuf0)
    b_project(2, slab0, slab1)
    b_output(0, obuf0)
    b_attend(1, slab1, obuf1)

    def p1_body(t, carry):
        @pl.when(t + AHEAD < NP)
        def _():
            start_pair(t + AHEAD)

        wait_pair(t - 1)
        k = 2 * t
        b_project(k + 1, slab1, slab0)
        b_output(k - 1, obuf1)
        b_attend(k, slab0, obuf0)
        a_weights(t - 1, (t - 1) % NSLOT)
        b_project(jnp.minimum(k + 2, NB - 1), slab0, slab1)
        b_output(k, obuf0)
        b_attend(k + 1, slab1, obuf1)
        return carry

    jax.lax.fori_loop(1, NP, p1_body, 0)
    wait_pair(NP - 1)
    b_output(NB - 1, obuf1)
    a_weights(NP - 1, (NP - 1) % NSLOT)

    h_ref[0:M, :] = mem_ref[...].astype(F32)
    gate = gate_ref[...].astype(F32).reshape(1, D)
    lag_b, lag_e, lag_f = 1, 3, 7

    def segment(s, carry):
        off = pl.multiple_of(s * SEG, SEG)
        x = xa_v[pl.ds(off, SEG), :].astype(F32)
        h_ref[M:L, :] = x
        r = jax.lax.broadcasted_iota(jnp.int32, (L, 2 * L), 0)
        c = jax.lax.broadcasted_iota(jnp.int32, (L, 2 * L), 1)
        isb = c >= L
        key = jnp.where(isb, c - L, c)
        allowed = (r < M) | (r >= key)
        st = [dict() for _ in range(NP)]
        acc = [None]

        def project(p):
            h = h_ref[...]
            b = p * 3 * PW
            st[p]['q'] = _dot(h, _w(w32[:, b:b + PW]))
            st[p]['kb'] = _blockdiag(_dot(h, _w(w32[:, b + PW:b + 2 * PW])))
            st[p]['vb'] = _blockdiag(_dot(h, _w(w32[:, b + 2 * PW:b + 3 * PW])))

        def softmax(p):
            sc = _dot(st[p].pop('q'), st[p].pop('kb'), NT)
            t = jnp.where(allowed, sc * (DH ** -0.5 * LOG2E), MASK_VALUE * LOG2E)
            ma = jnp.max(jnp.where(isb, -jnp.inf, t), axis=1, keepdims=True)
            mb = jnp.max(jnp.where(isb, t, -jnp.inf), axis=1, keepdims=True)
            e = jnp.exp2(t - jnp.where(isb, mb, ma))
            sa = jnp.sum(jnp.where(isb, 0.0, e), axis=1, keepdims=True)
            sb = jnp.sum(jnp.where(isb, e, 0.0), axis=1, keepdims=True)
            st[p]['p'] = e * _recip(jnp.where(isb, sb, sa))

        def values(p):
            st[p]['o'] = _dot(st[p].pop('p'), st[p].pop('vb'))

        def output(p):
            y = _dot(st[p].pop('o'), _w(wo32[p * (PW // 2):(p + 1) * (PW // 2), :]))
            acc[0] = y if acc[0] is None else acc[0] + y

        for t in range(NP + max(lag_b, lag_e, lag_f)):
            if t < NP:
                project(t)
            if 0 <= t - lag_b < NP:
                softmax(t - lag_b)
            if 0 <= t - lag_e < NP:
                values(t - lag_e)
            if 0 <= t - lag_f < NP:
                output(t - lag_f)
        a = acc[0]
        h_ref[0:M, :] = a[0:M]
        z = jnp.sum(x * gate, axis=1, keepdims=True)
        g = 1.0 / (1.0 + jnp.exp(-z))
        y = g * a[M:L] + (1.0 - g) * b_v[pl.ds(off, SEG), :]
        out_v[pl.ds(off, SEG), :] = y.astype(out_v.dtype)
        pltpu.make_async_copy(out_v.at[pl.ds(off, SEG), :], out_hbm.at[pl.ds(off, SEG), :],
                              sem_out.at[0]).start()
        return carry

    jax.lax.fori_loop(0, NSEG, segment, 0)
    pltpu.make_async_copy(out_v, out_hbm, sem_out.at[0]).wait()


@functools.partial(jax.jit, static_argnames=("A_seg_len",))
def pallas_gated_mix__memory_aug_recurrent_mem_tr__sliding_local_dilated__prompt_kernel(
    A_x: jax.Array,
    A_mem0: jax.Array,
    A_Wq: jax.Array,
    A_Wk: jax.Array,
    A_Wv: jax.Array,
    A_Wo: jax.Array,
    A_seg_len: int,
    B_x: jax.Array,
    B_wqkv: jax.Array,
    B_wo: jax.Array,
    gate_w: jax.Array,
):
    del B_x
    assert A_seg_len == SEG
    assert A_x.shape == (1, S, D) and A_Wq.shape == (D, H, DH) and A_mem0.shape == (1, M, D)

    def wt(w):
        return jnp.transpose(w, (1, 2, 0)).reshape(H * DH, D)

    hbm = pl.BlockSpec(memory_space=pl.ANY)
    vmem = pl.BlockSpec(memory_space=pltpu.VMEM)
    out = pl.pallas_call(
        _kernel,
        out_shape=jax.ShapeDtypeStruct((S, D), BF16),
        in_specs=[hbm, vmem, hbm, hbm, hbm, hbm, hbm, hbm, vmem],
        out_specs=hbm,
        scratch_shapes=[
            pltpu.VMEM((S, D), BF16),
            pltpu.VMEM((S, D), BF16),
            pltpu.VMEM((S, D), F32),
            pltpu.VMEM((L, D), F32),
            pltpu.VMEM((NSLOT, 4, PW, D), BF16),
            pltpu.VMEM((D // 2, 3 * H * DH), U32),
            pltpu.VMEM((H * DH // 2, D), U32),
            pltpu.VMEM((D, 3 * D), BF16),
            pltpu.VMEM((D, D), BF16),
            pltpu.VMEM((3 * D // 2, D), U32),
            pltpu.VMEM((D // 2, D), U32),
            pltpu.VMEM((NT_, 3 * D, 128), F32),
            pltpu.VMEM((3 * NT_, HALO + RB, 128), F32),
            pltpu.VMEM((3 * NT_, HALO + RB, 128), F32),
            pltpu.VMEM((RB, D), F32),
            pltpu.VMEM((RB, D), F32),
            pltpu.SemaphoreType.DMA((NP,)),
            pltpu.SemaphoreType.DMA((3,)),
            pltpu.SemaphoreType.DMA((1,)),
        ],
        compiler_params=pltpu.CompilerParams(vmem_limit_bytes=110 * 1024 * 1024,
                                             disable_bounds_checks=True),
    )(A_x.reshape(S, D), A_mem0.reshape(M, D), wt(A_Wq), wt(A_Wk), wt(A_Wv),
      A_Wo.reshape(H * DH, D), B_wqkv, B_wo, gate_w)
    return out.reshape(1, S, D)
```

```python
import functools

import jax
import jax.numpy as jnp
from jax.experimental import pallas as pl
from jax.experimental.pallas import tpu as pltpu

F32 = jnp.float32
BF16 = jnp.bfloat16
U32 = jnp.uint32

S = 2048
D = 640
H = 32
DH = 192
M = 8
SEG = 32
L = M + SEG
NSEG = S // SEG
NP = H // 2
PW = 2 * DH
MASK_VALUE = -1e9
LOG2E = 1.4426950408889634
HB = 32
DB = D // HB
WIN = 8
DIL = 2
RB = 64
NB = S // RB
HALO = 16
NT_ = D // 128


NN = (((1,), (0,)), ((), ()))
NT = (((1,), (1,)), ((), ()))


def _dot(a, b, dims=NN):
    return jax.lax.dot_general(a, b, dims, preferred_element_type=F32)


def _w(x):
    return pltpu.bitcast(x, BF16)


def _pack(x):
    return pltpu.bitcast(x, U32)


def _recip(den):
    r = pl.reciprocal(den, approx=True)
    return r * (2.0 - den * r)


def _blockdiag(t):
    lo = jax.lax.broadcasted_iota(jnp.int32, (L, 128), 1) < 64
    z = jnp.zeros((L, 128), F32)
    t0, t1, t2 = t[:, 0:128], t[:, 128:256], t[:, 256:384]
    top = jnp.concatenate([t0, jnp.where(lo, t1, 0.0), z], axis=1)
    bot = jnp.concatenate([z, jnp.where(lo, 0.0, t1), t2], axis=1)
    return jnp.concatenate([top, bot], axis=0).astype(BF16)


def _kernel(cfg, xa_hbm, mem_ref, wq_hbm, wk_hbm, wv_hbm, wo_hbm,
            wqkvb_hbm, wob_hbm, gate_ref,
            out_hbm,
            xa_v, out_v, b_v, h_ref,
            stage, w32, wo32,
            wqkvb_v, wob_v, wqkvb32, wob32, prep, slab0, slab1, obuf0, obuf1,
            sem_w, sem_in, sem_out):
    AHEAD = cfg.get('ahead', 4)
    NSLOT = cfg.get('nslot', 6)
    first = cfg.get('first', 0)
    def pair_copies(p, slot):
        rows = pl.ds(pl.multiple_of(p * PW, 128), PW)
        return [pltpu.make_async_copy(src.at[rows, :], stage.at[slot, i], sem_w.at[p])
                for i, src in enumerate((wq_hbm, wk_hbm, wv_hbm, wo_hbm))]

    c_wqkvb = pltpu.make_async_copy(wqkvb_hbm, wqkvb_v, sem_in.at[0])
    c_wob = pltpu.make_async_copy(wob_hbm, wob_v, sem_in.at[1])
    c_xa = pltpu.make_async_copy(xa_hbm, xa_v, sem_in.at[2])
    c_wqkvb.start()
    c_xa.start()
    c_wob.start()
    for p in range(first):
        if not cfg.get('nodma'):
            for c in pair_copies(p, p):
                c.start()

    c_wqkvb.wait()
    for p in range(first, AHEAD):
        if not cfg.get('nodma'):
            for c in pair_copies(p, p):
                c.start()
    for c in range(3 * NT_):
        t = wqkvb_v[:, c * 128:(c + 1) * 128].astype(F32).T
        for kt in range(NT_):
            prep[kt, c * 128:(c + 1) * 128, :] = t[:, kt * 128:(kt + 1) * 128]
    for part in range(3):
        for d in range(DB):
            rows = jnp.concatenate(
                [prep[kt, pl.ds(part * D + d, HB, stride=DB), :] for kt in range(NT_)], axis=1)
            r0 = (part * D + d * HB) // 2
            wqkvb32[r0:r0 + HB // 2, :] = _pack(rows.astype(BF16))
    c_wob.wait()
    for kt in range(NT_):
        prep[kt, 0:D, :] = wob_v[:, kt * 128:(kt + 1) * 128].astype(F32)
    for d in range(DB):
        rows = jnp.concatenate(
            [prep[kt, pl.ds(d, HB, stride=DB), :] for kt in range(NT_)], axis=1)
        wob32[d * (HB // 2):(d + 1) * (HB // 2), :] = _pack(rows.astype(BF16))

    def b_project(blk, dst, prev):
        if cfg.get('nob'):
            return
        x = xa_v[pl.ds(pl.multiple_of(blk * RB, RB), RB), :]
        for j in range(3 * NT_):
            dst[j, HALO:HALO + RB, :] = _dot(x, _w(wqkvb32[j * 64:(j + 1) * 64, :]), NT)
        for j in range(NT_, 3 * NT_):
            if prev is None:
                dst[j, 0:HALO, :] = jnp.zeros((HALO, 128), F32)
            else:
                dst[j, 0:HALO, :] = prev[j, RB:RB + HALO, :]

    def b_attend_rows(src, base, n, row0):
        q = [src[j, HALO + base:HALO + base + n, :] for j in range(NT_)]
        row = jax.lax.broadcasted_iota(jnp.int32, (n, 128), 0) + (row0 + base)
        logits = []
        for w in range(WIN):
            o = HALO + base - DIL * w
            s = q[0] * src[NT_, o:o + n, :]
            for j in range(1, NT_):
                s = s + q[j] * src[NT_ + j, o:o + n, :]
            s = s + pltpu.roll(s, 64, 1)
            s = s + pltpu.roll(s, 32, 1)
            s = s * (DB ** -0.5 * LOG2E)
            if w:
                s = jnp.where(row >= DIL * w, s, MASK_VALUE * LOG2E)
            logits.append(s)
        m = logits[0]
        for w in range(1, WIN):
            m = jnp.maximum(m, logits[w])
        e = [jnp.exp2(l - m) for l in logits]
        den = e[0]
        for w in range(1, WIN):
            den = den + e[w]
        r = _recip(den)
        outs = []
        for j in range(NT_):
            acc = None
            for w in range(WIN):
                o = HALO + base - DIL * w
                t = e[w] * src[2 * NT_ + j, o:o + n, :]
                acc = t if acc is None else acc + t
            outs.append(acc * r)
        return jnp.concatenate(outs, axis=1)

    def b_attend(blk, src, o_dst):
        if cfg.get('nob') or cfg.get('noattend'):
            return
        o_dst[...] = b_attend_rows(src, 0, RB, blk * RB)

    def b_output(blk, o_src):
        if cfg.get('nob'):
            return
        b_v[pl.ds(pl.multiple_of(blk * RB, RB), RB), :] = _dot(o_src[...], _w(wob32[...]))

    def a_weights(p, slot):
        if cfg.get('noxpose'):
            return
        col = pl.multiple_of(p * 3 * PW, 128)
        for i in range(3):
            w32[:, pl.ds(col + i * PW, PW)] = _pack(stage[slot, i].astype(F32).T.astype(BF16))
        wo32[pl.ds(pl.multiple_of(p * (PW // 2), 64), PW // 2), :] = _pack(stage[slot, 3])

    def start_pair(p):
        if cfg.get('nodma'):
            return
        for c in pair_copies(p, p % NSLOT):
            c.start()

    def wait_pair(p):
        if cfg.get('nodma'):
            return
        for c in pair_copies(p, p % NSLOT):
            c.wait()

    c_xa.wait()
    b_project(0, slab0, None)
    start_pair(AHEAD)
    b_project(1, slab1, slab0)
    b_attend(0, slab0, obuf0)
    b_project(2, slab0, slab1)
    b_output(0, obuf0)
    b_attend(1, slab1, obuf1)

    def p1_body(t, carry):
        @pl.when(t + AHEAD < NP)
        def _():
            start_pair(t + AHEAD)

        wait_pair(t - 1)
        k = 2 * t
        b_project(k + 1, slab1, slab0)
        b_output(k - 1, obuf1)
        b_attend(k, slab0, obuf0)
        a_weights(t - 1, (t - 1) % NSLOT)
        b_project(jnp.minimum(k + 2, NB - 1), slab0, slab1)
        b_output(k, obuf0)
        b_attend(k + 1, slab1, obuf1)
        return carry

    jax.lax.fori_loop(1, NP, p1_body, 0)
    wait_pair(NP - 1)
    b_output(NB - 1, obuf1)
    a_weights(NP - 1, (NP - 1) % NSLOT)

    h_ref[0:M, :] = mem_ref[...].astype(F32)
    gate = gate_ref[...].astype(F32).reshape(1, D)
    lag_b, lag_e, lag_f = 1, 3, 7

    def segment(s, carry):
        off = pl.multiple_of(s * SEG, SEG)
        x = xa_v[pl.ds(off, SEG), :].astype(F32)
        h_ref[M:L, :] = x
        r = jax.lax.broadcasted_iota(jnp.int32, (L, 2 * L), 0)
        c = jax.lax.broadcasted_iota(jnp.int32, (L, 2 * L), 1)
        isb = c >= L
        key = jnp.where(isb, c - L, c)
        allowed = (r < M) | (r >= key)
        st = [dict() for _ in range(NP)]
        acc = [None]

        def project(p):
            h = h_ref[...]
            b = p * 3 * PW
            st[p]['q'] = _dot(h, _w(w32[:, b:b + PW]))
            st[p]['kb'] = _blockdiag(_dot(h, _w(w32[:, b + PW:b + 2 * PW])))
            st[p]['vb'] = _blockdiag(_dot(h, _w(w32[:, b + 2 * PW:b + 3 * PW])))

        def softmax(p):
            sc = _dot(st[p].pop('q'), st[p].pop('kb'), NT)
            t = jnp.where(allowed, sc * (DH ** -0.5 * LOG2E), MASK_VALUE * LOG2E)
            ma = jnp.max(jnp.where(isb, -jnp.inf, t), axis=1, keepdims=True)
            mb = jnp.max(jnp.where(isb, t, -jnp.inf), axis=1, keepdims=True)
            e = jnp.exp2(t - jnp.where(isb, mb, ma))
            sa = jnp.sum(jnp.where(isb, 0.0, e), axis=1, keepdims=True)
            sb = jnp.sum(jnp.where(isb, e, 0.0), axis=1, keepdims=True)
            st[p]['p'] = e * _recip(jnp.where(isb, sb, sa))

        def values(p):
            st[p]['o'] = _dot(st[p].pop('p'), st[p].pop('vb'))

        def output(p):
            y = _dot(st[p].pop('o'), _w(wo32[p * (PW // 2):(p + 1) * (PW // 2), :]))
            acc[0] = y if acc[0] is None else acc[0] + y

        for t in range(NP + max(lag_b, lag_e, lag_f)):
            if t < NP:
                project(t)
            if 0 <= t - lag_b < NP:
                softmax(t - lag_b)
            if 0 <= t - lag_e < NP:
                values(t - lag_e)
            if 0 <= t - lag_f < NP:
                output(t - lag_f)
        a = acc[0]
        h_ref[0:M, :] = a[0:M]
        z = jnp.sum(x * gate, axis=1, keepdims=True)
        g = 1.0 / (1.0 + jnp.exp(-z))
        y = g * a[M:L] + (1.0 - g) * b_v[pl.ds(off, SEG), :]
        out_v[pl.ds(off, SEG), :] = y.astype(out_v.dtype)
        pltpu.make_async_copy(out_v.at[pl.ds(off, SEG), :], out_hbm.at[pl.ds(off, SEG), :],
                              sem_out.at[0]).start()
        return carry

    nseg = cfg.get('nseg', NSEG)
    if nseg == 0:
        return
    jax.lax.fori_loop(0, nseg, segment, 0)
    pltpu.make_async_copy(out_v.at[0:nseg * SEG, :], out_hbm.at[0:nseg * SEG, :], sem_out.at[0]).wait()


def _forward(cfg, A_x, A_mem0, A_Wq, A_Wk, A_Wv, A_Wo, B_wqkv, B_wo, gate_w):
    def wt(w):
        return jnp.transpose(w, (1, 2, 0)).reshape(H * DH, D)

    hbm = pl.BlockSpec(memory_space=pl.ANY)
    vmem = pl.BlockSpec(memory_space=pltpu.VMEM)
    out = pl.pallas_call(
        functools.partial(_kernel, cfg),
        out_shape=jax.ShapeDtypeStruct((S, D), BF16),
        in_specs=[hbm, vmem, hbm, hbm, hbm, hbm, hbm, hbm, vmem],
        out_specs=hbm,
        scratch_shapes=[
            pltpu.VMEM((S, D), BF16),
            pltpu.VMEM((S, D), BF16),
            pltpu.VMEM((S, D), F32),
            pltpu.VMEM((L, D), F32),
            pltpu.VMEM((cfg.get('nslot', 6), 4, PW, D), BF16),
            pltpu.VMEM((D // 2, 3 * H * DH), U32),
            pltpu.VMEM((H * DH // 2, D), U32),
            pltpu.VMEM((D, 3 * D), BF16),
            pltpu.VMEM((D, D), BF16),
            pltpu.VMEM((3 * D // 2, D), U32),
            pltpu.VMEM((D // 2, D), U32),
            pltpu.VMEM((NT_, 3 * D, 128), F32),
            pltpu.VMEM((3 * NT_, HALO + RB, 128), F32),
            pltpu.VMEM((3 * NT_, HALO + RB, 128), F32),
            pltpu.VMEM((RB, D), F32),
            pltpu.VMEM((RB, D), F32),
            pltpu.SemaphoreType.DMA((NP,)),
            pltpu.SemaphoreType.DMA((3,)),
            pltpu.SemaphoreType.DMA((1,)),
        ],
        compiler_params=pltpu.CompilerParams(vmem_limit_bytes=110 * 1024 * 1024,
                                             disable_bounds_checks=True),
    )(A_x.reshape(S, D), A_mem0.reshape(M, D), wt(A_Wq), wt(A_Wk), wt(A_Wv),
      A_Wo.reshape(H * DH, D), B_wqkv, B_wo, gate_w)
    return out.reshape(1, S, D)


@functools.partial(jax.jit, static_argnames=("A_seg_len",))
def pallas_gated_mix__memory_aug_recurrent_mem_tr__sliding_local_dilated__prompt_kernel(
    A_x: jax.Array,
    A_mem0: jax.Array,
    A_Wq: jax.Array,
    A_Wk: jax.Array,
    A_Wv: jax.Array,
    A_Wo: jax.Array,
    A_seg_len: int,
    B_x: jax.Array,
    B_wqkv: jax.Array,
    B_wo: jax.Array,
    gate_w: jax.Array,
):
    del B_x
    assert A_seg_len == SEG
    assert A_x.shape == (1, S, D) and A_Wq.shape == (D, H, DH) and A_mem0.shape == (1, M, D)
    return _forward({}, A_x, A_mem0, A_Wq, A_Wk, A_Wv, A_Wo, B_wqkv, B_wo, gate_w)
```

```python
import functools

import jax
import jax.numpy as jnp
from jax.experimental import pallas as pl
from jax.experimental.pallas import tpu as pltpu

F32 = jnp.float32
BF16 = jnp.bfloat16
U32 = jnp.uint32

S = 2048
D = 640
H = 32
DH = 192
M = 8
SEG = 32
L = M + SEG
NSEG = S // SEG
NP = H // 2
PW = 2 * DH
MASK_VALUE = -1e9
LOG2E = 1.4426950408889634
HB = 32
DB = D // HB
WIN = 8
DIL = 2
RB = 128
XA0 = 256
NB = S // RB
HALO = 16
NT_ = D // 128


NN = (((1,), (0,)), ((), ()))
NT = (((1,), (1,)), ((), ()))


def _dot(a, b, dims=NN):
    return jax.lax.dot_general(a, b, dims, preferred_element_type=F32)


def _w(x):
    return pltpu.bitcast(x, BF16)


def _pack(x):
    return pltpu.bitcast(x, U32)


def _recip(den):
    r = pl.reciprocal(den, approx=True)
    return r * (2.0 - den * r)


def _blockdiag(t):
    lo = jax.lax.broadcasted_iota(jnp.int32, (L, 128), 1) < 64
    z = jnp.zeros((L, 128), F32)
    t0, t1, t2 = t[:, 0:128], t[:, 128:256], t[:, 256:384]
    top = jnp.concatenate([t0, jnp.where(lo, t1, 0.0), z], axis=1)
    bot = jnp.concatenate([z, jnp.where(lo, 0.0, t1), t2], axis=1)
    return jnp.concatenate([top, bot], axis=0).astype(BF16)


def _kernel(cfg, xa_hbm, mem_ref, wq_hbm, wk_hbm, wv_hbm, wo_hbm,
            wqkvb_hbm, wob_hbm, gate_ref,
            out_hbm,
            xa_v, out_v, b_v, h_ref,
            stage, wo_stage, w32, wo32,
            wqkvb_v, wob_v, wqkvb32, wob32, prep, fresh, cur, onew, ocur, x32,
            sem_qkv, sem_in, sem_out):
    def qkv_copies(p):
        rows = pl.ds(pl.multiple_of(p * PW, 128), PW)
        return [pltpu.make_async_copy(src.at[rows, :], stage.at[i, rows, :], sem_qkv.at[p])
                for i, src in enumerate((wq_hbm, wk_hbm, wv_hbm))]

    c_wo = pltpu.make_async_copy(wo_hbm, wo_stage, sem_in.at[4])
    c_wqkvb = pltpu.make_async_copy(wqkvb_hbm, wqkvb_v, sem_in.at[0])
    c_wob = pltpu.make_async_copy(wob_hbm, wob_v, sem_in.at[1])
    c_xa0 = pltpu.make_async_copy(xa_hbm.at[0:XA0, :], xa_v.at[0:XA0, :], sem_in.at[2])
    c_xa1 = pltpu.make_async_copy(xa_hbm.at[XA0:S, :], xa_v.at[XA0:S, :], sem_in.at[3])
    c_wqkvb.start()
    c_xa0.start()
    c_wob.start(priority=1)
    c_xa1.start(priority=1)

    c_wqkvb.wait()
    if not cfg.get('nodma'):
        for p in range(NP):
            for c in qkv_copies(p):
                c.start(priority=cfg.get('prio', 1))
    for c in range(3 * NT_):
        t = wqkvb_v[:, c * 128:(c + 1) * 128].astype(F32).T
        for kt in range(NT_):
            prep[kt, c * 128:(c + 1) * 128, :] = t[:, kt * 128:(kt + 1) * 128]
    for part in range(3):
        for d in range(DB):
            rows = jnp.concatenate(
                [prep[kt, pl.ds(part * D + d, HB, stride=DB), :] for kt in range(NT_)], axis=1)
            r0 = (part * D + d * HB) // 2
            wqkvb32[r0:r0 + HB // 2, :] = _pack(rows.astype(BF16))

    def prep_wob():
        for kt in range(NT_):
            prep[kt, 0:D, :] = wob_v[:, kt * 128:(kt + 1) * 128].astype(F32)
        for d in range(DB):
            rows = jnp.concatenate(
                [prep[kt, pl.ds(d, HB, stride=DB), :] for kt in range(NT_)], axis=1)
            wob32[d * (HB // 2):(d + 1) * (HB // 2), :] = _pack(rows.astype(BF16))

    def b_project(blk, first=False):
        x = xa_v[pl.ds(pl.multiple_of(blk * RB, RB), RB), :]
        xp = x32.at[1 if first else 0]
        xp[...] = _pack(x)
        for j in range(3 * NT_):
            x = _w(xp[...])
            y = _dot(x, _w(wqkvb32[j * 64:(j + 1) * 64, :]), NT)
            if first:
                cur[j, HALO:HALO + RB, :] = y
                if j >= NT_:
                    cur[j, 0:HALO, :] = jnp.zeros((HALO, 128), F32)
            else:
                fresh[j] = y

    def b_rotate():
        for j in range(NT_, 3 * NT_):
            cur[j, 0:HALO, :] = cur[j, RB:RB + HALO, :]
        for j in range(3 * NT_):
            cur[j, HALO:HALO + RB, :] = fresh[j]
        ocur[...] = onew[...]

    def b_attend_rows(base, n, row0):
        src = cur
        q = [src[j, HALO + base:HALO + base + n, :] for j in range(NT_)]
        row = jax.lax.broadcasted_iota(jnp.int32, (n, 128), 0) + (row0 + base)
        half = WIN // 2
        step = DIL * half
        logits = [None] * WIN
        for w in range(half):
            o = HALO + base - DIL * w - step
            lo = hi = None
            for j in range(NT_):
                k = src[NT_ + j, o:o + n + step, :]
                a, b = q[j] * k[step:], q[j] * k[:n]
                lo = a if lo is None else lo + a
                hi = b if hi is None else hi + b
            for ww, s in ((w, lo), (w + half, hi)):
                s = s + pltpu.roll(s, 64, 1)
                s = s + pltpu.roll(s, 32, 1)
                s = s * (DB ** -0.5 * LOG2E)
                if ww:
                    s = jnp.where(row >= DIL * ww, s, MASK_VALUE * LOG2E)
                logits[ww] = s
        m = logits[0]
        for w in range(1, WIN):
            m = jnp.maximum(m, logits[w])
        e = [jnp.exp2(l - m) for l in logits]
        den = e[0]
        for w in range(1, WIN):
            den = den + e[w]
        r = _recip(den)
        outs = []
        for j in range(NT_):
            acc = None
            for w in range(half):
                o = HALO + base - DIL * w - step
                v = src[2 * NT_ + j, o:o + n + step, :]
                t = e[w] * v[step:] + e[w + half] * v[:n]
                acc = t if acc is None else acc + t
            outs.append(acc * r)
        return jnp.concatenate(outs, axis=1)

    def b_attend(blk, between=()):
        sub = cfg.get('sub', 64)
        between = list(between)
        for base in range(0, RB, sub):
            if between:
                between.pop(0)()
            onew[base:base + sub, :] = b_attend_rows(base, sub, blk * RB)
        for f in between:
            f()

    def b_output(blk, src):
        b_v[pl.ds(pl.multiple_of(blk * RB, RB), RB), :] = _dot(src[...], _w(wob32[...]))

    def qkv_weight(p, i):
        if cfg.get('nodma'):
            return
        rows = pl.ds(pl.multiple_of(p * PW, 128), PW)
        col = pl.multiple_of(p * 3 * PW, 128)
        w32[:, pl.ds(col + i * PW, PW)] = _pack(stage[i, rows, :].astype(F32).T.astype(BF16))

    def qkv_weights(p):
        for i in range(3):
            qkv_weight(p, i)

    def wait_qkv(p):
        if cfg.get('nodma'):
            return
        for c in qkv_copies(p):
            c.wait()

    c_wob.wait()
    c_xa0.wait()
    b_project(0, first=True)
    if not cfg.get('nodma'):
        c_wo.start(priority=cfg.get('prio', 1))
    if cfg.get('wob_pos', 2) == 0:
        prep_wob()
    b_project(1)
    if cfg.get('wob_pos', 2) == 1:
        prep_wob()
    b_attend(0)
    if cfg.get('wob_pos', 2) == 2:
        prep_wob()
    b_rotate()
    c_xa1.wait()

    def p1_body(k, carry):
        wait_qkv(k - 1)
        for c in cfg.get('order', 'poatr'):
            if c == 'p':
                b_project(k + 1)
            elif c == 'o':
                b_output(k - 1, ocur)
            elif c == 'a':
                b_attend(k)
            elif c == 't':
                qkv_weights(k - 1)
            elif c == 'r':
                b_rotate()
        return carry

    jax.lax.fori_loop(1, NB - 1, p1_body, 0)
    wait_qkv(NB - 2)
    wait_qkv(NB - 1)
    b_output(NB - 2, ocur)
    if cfg.get('batt_t', 0) < 0:
        b_attend(NB - 1)
    qkv_weights(NB - 2)
    qkv_weights(NB - 1)

    h_ref[0:M, :] = mem_ref[...].astype(F32)
    gate = gate_ref[...].astype(F32).reshape(1, D)
    lag_b, lag_e, lag_f = 1, 3, 7

    def segment(s, carry, first=False):
        off = s * SEG if first else pl.multiple_of(s * SEG, SEG)
        x = xa_v[pl.ds(off, SEG), :].astype(F32)
        h_ref[M:L, :] = x
        r = jax.lax.broadcasted_iota(jnp.int32, (L, 2 * L), 0)
        c = jax.lax.broadcasted_iota(jnp.int32, (L, 2 * L), 1)
        isb = c >= L
        key = jnp.where(isb, c - L, c)
        allowed = (r < M) | (r >= key)
        st = [dict() for _ in range(NP)]
        acc = [None]

        def project(p):
            h = h_ref[...]
            b = p * 3 * PW
            st[p]['q'] = _dot(h, _w(w32[:, b:b + PW]))
            st[p]['kb'] = _blockdiag(_dot(h, _w(w32[:, b + PW:b + 2 * PW])))
            st[p]['vb'] = _blockdiag(_dot(h, _w(w32[:, b + 2 * PW:b + 3 * PW])))

        def softmax(p):
            sc = _dot(st[p].pop('q'), st[p].pop('kb'), NT)
            t = jnp.where(allowed, sc * (DH ** -0.5 * LOG2E), MASK_VALUE * LOG2E)
            ma = jnp.max(jnp.where(isb, -jnp.inf, t), axis=1, keepdims=True)
            mb = jnp.max(jnp.where(isb, t, -jnp.inf), axis=1, keepdims=True)
            e = jnp.exp2(t - jnp.where(isb, mb, ma))
            sa = jnp.sum(jnp.where(isb, 0.0, e), axis=1, keepdims=True)
            sb = jnp.sum(jnp.where(isb, e, 0.0), axis=1, keepdims=True)
            st[p]['p'] = e * _recip(jnp.where(isb, sb, sa))

        def values(p):
            st[p]['o'] = _dot(st[p].pop('p'), st[p].pop('vb'))

        def output(p):
            if first:
                w = wo_stage[p * PW:(p + 1) * PW, :]
                wo32[p * (PW // 2):(p + 1) * (PW // 2), :] = _pack(w)
            else:
                w = _w(wo32[p * (PW // 2):(p + 1) * (PW // 2), :])
            y = _dot(st[p].pop('o'), w)
            acc[0] = y if acc[0] is None else acc[0] + y

        for t in range(NP + max(lag_b, lag_e, lag_f)):
            if t < NP:
                project(t)
            if first and t == cfg.get('batt_t', 0):
                b_attend(NB - 1)
            if first and t == cfg.get('bout_t', 16):
                b_output(NB - 1, onew)
            if 0 <= t - lag_b < NP:
                softmax(t - lag_b)
            if 0 <= t - lag_e < NP:
                values(t - lag_e)
            if not first and 0 <= t - lag_f < NP:
                output(t - lag_f)
        if first:
            if not cfg.get('nodma'):
                c_wo.wait()
            for p in range(NP):
                output(p)
        a = acc[0]
        h_ref[0:M, :] = a[0:M]
        z = jnp.sum(x * gate, axis=1, keepdims=True)
        g = 1.0 / (1.0 + jnp.exp(-z))
        y = g * a[M:L] + (1.0 - g) * b_v[pl.ds(off, SEG), :]
        out_v[pl.ds(off, SEG), :] = y.astype(out_v.dtype)
        pltpu.make_async_copy(out_v.at[pl.ds(off, SEG), :], out_hbm.at[pl.ds(off, SEG), :],
                              sem_out.at[0]).start()
        return carry

    nseg = cfg.get('nseg', NSEG)
    if cfg.get('peel', True):
        segment(0, 0, first=True)
        start = 1
    else:
        b_attend(NB - 1)
        b_output(NB - 1, onew)
        c_wo.wait()
        for p in range(NP):
            wo32[p * (PW // 2):(p + 1) * (PW // 2), :] = _pack(wo_stage[p * PW:(p + 1) * PW, :])
        start = 0
    if nseg > start:
        jax.lax.fori_loop(start, nseg, segment, 0)
    n_out = max(nseg, start)
    if n_out:
        pltpu.make_async_copy(out_v.at[0:n_out * SEG, :], out_hbm.at[0:n_out * SEG, :],
                              sem_out.at[0]).wait()


def _forward(cfg, A_x, A_mem0, A_Wq, A_Wk, A_Wv, A_Wo, B_wqkv, B_wo, gate_w):
    def wt(w):
        return jnp.transpose(w, (1, 2, 0)).reshape(H * DH, D)

    hbm = pl.BlockSpec(memory_space=pl.ANY)
    vmem = pl.BlockSpec(memory_space=pltpu.VMEM)
    out = pl.pallas_call(
        functools.partial(_kernel, cfg),
        out_shape=jax.ShapeDtypeStruct((S, D), BF16),
        in_specs=[hbm, vmem, hbm, hbm, hbm, hbm, hbm, hbm, vmem],
        out_specs=hbm,
        scratch_shapes=[
            pltpu.VMEM((S, D), BF16),
            pltpu.VMEM((S, D), BF16),
            pltpu.VMEM((S, D), F32),
            pltpu.VMEM((L, D), F32),
            pltpu.VMEM((3, H * DH, D), BF16),
            pltpu.VMEM((H * DH, D), BF16),
            pltpu.VMEM((D // 2, 3 * H * DH), U32),
            pltpu.VMEM((H * DH // 2, D), U32),
            pltpu.VMEM((D, 3 * D), BF16),
            pltpu.VMEM((D, D), BF16),
            pltpu.VMEM((3 * D // 2, D), U32),
            pltpu.VMEM((D // 2, D), U32),
            pltpu.VMEM((NT_, 3 * D, 128), F32),
            pltpu.VMEM((3 * NT_, RB, 128), F32),
            pltpu.VMEM((3 * NT_, HALO + RB, 128), F32),
            pltpu.VMEM((RB, D), F32),
            pltpu.VMEM((RB, D), F32),
            pltpu.VMEM((2, RB // 2, D), U32),
            pltpu.SemaphoreType.DMA((NP,)),
            pltpu.SemaphoreType.DMA((5,)),
            pltpu.SemaphoreType.DMA((1,)),
        ],
        compiler_params=pltpu.CompilerParams(vmem_limit_bytes=120 * 1024 * 1024,
                                             disable_bounds_checks=True),
    )(A_x.reshape(S, D), A_mem0.reshape(M, D), wt(A_Wq), wt(A_Wk), wt(A_Wv),
      A_Wo.reshape(H * DH, D), B_wqkv, B_wo, gate_w)
    return out.reshape(1, S, D)


@functools.partial(jax.jit, static_argnames=("A_seg_len",))
def pallas_gated_mix__memory_aug_recurrent_mem_tr__sliding_local_dilated__prompt_kernel(
    A_x: jax.Array,
    A_mem0: jax.Array,
    A_Wq: jax.Array,
    A_Wk: jax.Array,
    A_Wv: jax.Array,
    A_Wo: jax.Array,
    A_seg_len: int,
    B_x: jax.Array,
    B_wqkv: jax.Array,
    B_wo: jax.Array,
    gate_w: jax.Array,
):
    del B_x
    assert A_seg_len == SEG
    assert A_x.shape == (1, S, D) and A_Wq.shape == (D, H, DH) and A_mem0.shape == (1, M, D)
    return _forward({}, A_x, A_mem0, A_Wq, A_Wk, A_Wv, A_Wo, B_wqkv, B_wo, gate_w)
```

```python
import functools

import jax
import jax.numpy as jnp
from jax.experimental import pallas as pl
from jax.experimental.pallas import tpu as pltpu

F32 = jnp.float32
BF16 = jnp.bfloat16
U32 = jnp.uint32

S = 2048
D = 640
H = 32
DH = 192
M = 8
SEG = 32
L = M + SEG
NSEG = S // SEG
NP = H // 2
PW = 2 * DH
MASK_VALUE = -1e9
LOG2E = 1.4426950408889634
HB = 32
DB = D // HB
WIN = 8
DIL = 2
RB = 128
XA0 = 256
NB = S // RB
HALO = 16
NT_ = D // 128


NN = (((1,), (0,)), ((), ()))
NT = (((1,), (1,)), ((), ()))


def _dot(a, b, dims=NN):
    return jax.lax.dot_general(a, b, dims, preferred_element_type=F32)


def _w(x):
    return pltpu.bitcast(x, BF16)


def _pack(x):
    return pltpu.bitcast(x, U32)


def _recip(den):
    r = pl.reciprocal(den, approx=True)
    return r * (2.0 - den * r)


def _blockdiag(t):
    lo = jax.lax.broadcasted_iota(jnp.int32, (L, 128), 1) < 64
    z = jnp.zeros((L, 128), F32)
    t0, t1, t2 = t[:, 0:128], t[:, 128:256], t[:, 256:384]
    top = jnp.concatenate([t0, jnp.where(lo, t1, 0.0), z], axis=1)
    bot = jnp.concatenate([z, jnp.where(lo, 0.0, t1), t2], axis=1)
    return jnp.concatenate([top, bot], axis=0).astype(BF16)


def _kernel(cfg, xa_hbm, mem_ref, wq_hbm, wk_hbm, wv_hbm, wo_hbm,
            wqkvb_hbm, wob_hbm, gate_ref,
            out_hbm,
            xa_v, out_v, b_v, h_ref,
            stage, wo_stage, w32, wo32,
            wqkvb_v, wob_v, wqkvb32, wob32, prep, fresh, cur, onew, ocur, x32,
            sem_qkv, sem_in, sem_out):
    def qkv_copies(p):
        rows = pl.ds(pl.multiple_of(p * PW, 128), PW)
        return [pltpu.make_async_copy(src.at[rows, :], stage.at[i, rows, :], sem_qkv.at[p])
                for i, src in enumerate((wq_hbm, wk_hbm, wv_hbm))]

    nwo = cfg.get('nwo', 1)
    wo_rows = H * DH // nwo
    c_wo = [pltpu.make_async_copy(wo_hbm.at[i * wo_rows:(i + 1) * wo_rows, :],
                                  wo_stage.at[i * wo_rows:(i + 1) * wo_rows, :], sem_in.at[4 + i])
            for i in range(nwo)]
    c_wqkvb = pltpu.make_async_copy(wqkvb_hbm, wqkvb_v, sem_in.at[0])
    c_wob = pltpu.make_async_copy(wob_hbm, wob_v, sem_in.at[1])
    c_xa0 = pltpu.make_async_copy(xa_hbm.at[0:XA0, :], xa_v.at[0:XA0, :], sem_in.at[2])
    c_xa1 = pltpu.make_async_copy(xa_hbm.at[XA0:S, :], xa_v.at[XA0:S, :], sem_in.at[3])
    c_wqkvb.start()
    c_xa0.start()
    c_wob.start(priority=1)
    c_xa1.start(priority=1)

    c_wqkvb.wait()
    if not cfg.get('nodma'):
        for p in range(NP):
            for c in qkv_copies(p):
                c.start(priority=cfg.get('prio', 1))
    for c in range(3 * NT_):
        t = wqkvb_v[:, c * 128:(c + 1) * 128].astype(F32).T
        for kt in range(NT_):
            prep[kt, c * 128:(c + 1) * 128, :] = t[:, kt * 128:(kt + 1) * 128]
    for part in range(3):
        for d in range(DB):
            rows = jnp.concatenate(
                [prep[kt, pl.ds(part * D + d, HB, stride=DB), :] for kt in range(NT_)], axis=1)
            r0 = (part * D + d * HB) // 2
            wqkvb32[r0:r0 + HB // 2, :] = _pack(rows.astype(BF16))

    def prep_wob():
        for kt in range(NT_):
            prep[kt, 0:D, :] = wob_v[:, kt * 128:(kt + 1) * 128].astype(F32)
        for d in range(DB):
            rows = jnp.concatenate(
                [prep[kt, pl.ds(d, HB, stride=DB), :] for kt in range(NT_)], axis=1)
            wob32[d * (HB // 2):(d + 1) * (HB // 2), :] = _pack(rows.astype(BF16))

    def b_project(blk, first=False):
        x = xa_v[pl.ds(pl.multiple_of(blk * RB, RB), RB), :]
        xp = x32.at[1 if first else 0]
        xp[...] = _pack(x)
        for j in range(3 * NT_):
            x = _w(xp[...])
            y = _dot(x, _w(wqkvb32[j * 64:(j + 1) * 64, :]), NT)
            if first:
                cur[j, HALO:HALO + RB, :] = y
                if j >= NT_:
                    cur[j, 0:HALO, :] = jnp.zeros((HALO, 128), F32)
            else:
                fresh[j] = y

    def b_rotate():
        for j in range(NT_, 3 * NT_):
            cur[j, 0:HALO, :] = cur[j, RB:RB + HALO, :]
        for j in range(3 * NT_):
            cur[j, HALO:HALO + RB, :] = fresh[j]
        ocur[...] = onew[...]

    def b_attend_rows(base, n, row0):
        src = cur
        q = [src[j, HALO + base:HALO + base + n, :] for j in range(NT_)]
        row = jax.lax.broadcasted_iota(jnp.int32, (n, 128), 0) + (row0 + base)
        half = WIN // 2
        step = DIL * half
        logits = [None] * WIN
        for w in range(half):
            o = HALO + base - DIL * w - step
            lo = hi = None
            for j in range(NT_):
                k = src[NT_ + j, o:o + n + step, :]
                a, b = q[j] * k[step:], q[j] * k[:n]
                lo = a if lo is None else lo + a
                hi = b if hi is None else hi + b
            for ww, s in ((w, lo), (w + half, hi)):
                s = s + pltpu.roll(s, 64, 1)
                s = s + pltpu.roll(s, 32, 1)
                s = s * (DB ** -0.5 * LOG2E)
                if ww:
                    s = jnp.where(row >= DIL * ww, s, MASK_VALUE * LOG2E)
                logits[ww] = s
        m = logits[0]
        for w in range(1, WIN):
            m = jnp.maximum(m, logits[w])
        e = [jnp.exp2(l - m) for l in logits]
        den = e[0]
        for w in range(1, WIN):
            den = den + e[w]
        r = _recip(den)
        outs = []
        for j in range(NT_):
            acc = None
            for w in range(half):
                o = HALO + base - DIL * w - step
                v = src[2 * NT_ + j, o:o + n + step, :]
                t = e[w] * v[step:] + e[w + half] * v[:n]
                acc = t if acc is None else acc + t
            outs.append(acc * r)
        return jnp.concatenate(outs, axis=1)

    def b_attend(blk, between=()):
        sub = cfg.get('sub', 64)
        between = list(between)
        for base in range(0, RB, sub):
            if between:
                between.pop(0)()
            onew[base:base + sub, :] = b_attend_rows(base, sub, blk * RB)
        for f in between:
            f()

    def b_output(blk, src):
        b_v[pl.ds(pl.multiple_of(blk * RB, RB), RB), :] = _dot(src[...], _w(wob32[...]))

    def qkv_weight(p, i):
        if cfg.get('nodma'):
            return
        rows = pl.ds(pl.multiple_of(p * PW, 128), PW)
        col = pl.multiple_of(p * 3 * PW, 128)
        w32[:, pl.ds(col + i * PW, PW)] = _pack(stage[i, rows, :].astype(F32).T.astype(BF16))

    def qkv_weights(p):
        for i in range(3):
            qkv_weight(p, i)

    def wait_qkv(p):
        if cfg.get('nodma'):
            return
        for c in qkv_copies(p):
            c.wait()

    c_wob.wait()
    c_xa0.wait()
    b_project(0, first=True)
    if not cfg.get('nodma'):
        for c in c_wo:
            c.start(priority=1)
    if cfg.get('wob_pos', 2) == 0:
        prep_wob()
    b_project(1)
    if cfg.get('wob_pos', 2) == 1:
        prep_wob()
    b_attend(0)
    if cfg.get('wob_pos', 2) == 2:
        prep_wob()
    b_rotate()
    c_xa1.wait()

    def p1_step(k):
        for c in cfg.get('order', 'poatr'):
            if c == 'p':
                b_project(k + 1)
            elif c == 'o':
                b_output(k - 1, ocur)
            elif c == 'a':
                b_attend(k)
            elif c == 't':
                qkv_weights(k - 1)
            elif c == 'r':
                b_rotate()

    unroll = cfg.get('unroll', 1)

    def p1_body(i, carry):
        k0 = 1 + unroll * i
        for u in range(unroll):
            wait_qkv(k0 + u - 1)
        for u in range(unroll):
            p1_step(k0 + u)
        return carry

    jax.lax.fori_loop(0, (NB - 2) // unroll, p1_body, 0)
    wait_qkv(NB - 2)
    wait_qkv(NB - 1)
    b_output(NB - 2, ocur)
    if cfg.get('batt_t', 0) < 0:
        b_attend(NB - 1)
    qkv_weights(NB - 2)
    qkv_weights(NB - 1)

    h_ref[0:M, :] = mem_ref[...].astype(F32)
    gate = gate_ref[...].astype(F32).reshape(1, D)
    lag_b, lag_e, lag_f = cfg.get('lags', (1, 4, 8))

    def segment(s, carry, first=False):
        off = s * SEG if first else pl.multiple_of(s * SEG, SEG)
        x = xa_v[pl.ds(off, SEG), :].astype(F32)
        h_ref[M:L, :] = x
        r = jax.lax.broadcasted_iota(jnp.int32, (L, 2 * L), 0)
        c = jax.lax.broadcasted_iota(jnp.int32, (L, 2 * L), 1)
        isb = c >= L
        key = jnp.where(isb, c - L, c)
        allowed = (r < M) | (r >= key)
        st = [dict() for _ in range(NP)]
        acc = [None]

        def project(p):
            h = h_ref[...]
            b = p * 3 * PW
            st[p]['q'] = _dot(h, _w(w32[:, b:b + PW]))
            st[p]['kb'] = _blockdiag(_dot(h, _w(w32[:, b + PW:b + 2 * PW])))
            st[p]['vb'] = _blockdiag(_dot(h, _w(w32[:, b + 2 * PW:b + 3 * PW])))

        def softmax(p):
            sc = _dot(st[p].pop('q'), st[p].pop('kb'), NT)
            t = jnp.where(allowed, sc * (DH ** -0.5 * LOG2E), MASK_VALUE * LOG2E)
            ma = jnp.max(jnp.where(isb, -jnp.inf, t), axis=1, keepdims=True)
            mb = jnp.max(jnp.where(isb, t, -jnp.inf), axis=1, keepdims=True)
            e = jnp.exp2(t - jnp.where(isb, mb, ma))
            sa = jnp.sum(jnp.where(isb, 0.0, e), axis=1, keepdims=True)
            sb = jnp.sum(jnp.where(isb, e, 0.0), axis=1, keepdims=True)
            st[p]['p'] = e * _recip(jnp.where(isb, sb, sa))

        def values(p):
            st[p]['o'] = _dot(st[p].pop('p'), st[p].pop('vb'))

        def output(p):
            if first:
                w = wo_stage[p * PW:(p + 1) * PW, :]
                wo32[p * (PW // 2):(p + 1) * (PW // 2), :] = _pack(w)
            else:
                w = _w(wo32[p * (PW // 2):(p + 1) * (PW // 2), :])
            y = _dot(st[p].pop('o'), w)
            acc[0] = y if acc[0] is None else acc[0] + y

        nsteps = NP + (lag_e + 1 if first else lag_f)
        wo_t = cfg.get('wo_t', (nsteps - 1,))
        for t in range(nsteps):
            if t < NP:
                project(t)
            if first and t == cfg.get('batt_t', 0):
                b_attend(NB - 1)
            if first and t == cfg.get('bout_t', 16):
                b_output(NB - 1, onew)
            if 0 <= t - lag_b < NP:
                softmax(t - lag_b)
            if 0 <= t - lag_e < NP:
                values(t - lag_e)
            if not first and 0 <= t - lag_f < NP:
                output(t - lag_f)
            if first:
                for i, tw in enumerate(wo_t):
                    if t == tw and not cfg.get('nodma'):
                        c_wo[i].wait()
                    if t >= tw:
                        lo, hi = i * NP // nwo, (i + 1) * NP // nwo
                        per = -(-(hi - lo) // (nsteps - tw)) if tw < nsteps else hi - lo
                        for p in range(lo + (t - tw) * per, min(hi, lo + (t - tw + 1) * per)):
                            output(p)
        a = acc[0]
        h_ref[0:M, :] = a[0:M]
        z = jnp.sum(x * gate, axis=1, keepdims=True)
        g = 1.0 / (1.0 + jnp.exp(-z))
        y = g * a[M:L] + (1.0 - g) * b_v[pl.ds(off, SEG), :]
        out_v[pl.ds(off, SEG), :] = y.astype(out_v.dtype)
        pltpu.make_async_copy(out_v.at[pl.ds(off, SEG), :], out_hbm.at[pl.ds(off, SEG), :],
                              sem_out.at[0]).start()
        return carry

    nseg = cfg.get('nseg', NSEG)
    if cfg.get('peel', True):
        segment(0, 0, first=True)
        start = 1
    else:
        b_attend(NB - 1)
        b_output(NB - 1, onew)
        for c in c_wo:
            c.wait()
        for p in range(NP):
            wo32[p * (PW // 2):(p + 1) * (PW // 2), :] = _pack(wo_stage[p * PW:(p + 1) * PW, :])
        start = 0
    if nseg > start:
        jax.lax.fori_loop(start, nseg, segment, 0)
    n_out = max(nseg, start)
    if n_out:
        pltpu.make_async_copy(out_v.at[0:n_out * SEG, :], out_hbm.at[0:n_out * SEG, :],
                              sem_out.at[0]).wait()


def _forward(cfg, A_x, A_mem0, A_Wq, A_Wk, A_Wv, A_Wo, B_wqkv, B_wo, gate_w):
    def wt(w):
        return jnp.transpose(w, (1, 2, 0)).reshape(H * DH, D)

    hbm = pl.BlockSpec(memory_space=pl.ANY)
    vmem = pl.BlockSpec(memory_space=pltpu.VMEM)
    out = pl.pallas_call(
        functools.partial(_kernel, cfg),
        out_shape=jax.ShapeDtypeStruct((S, D), BF16),
        in_specs=[hbm, vmem, hbm, hbm, hbm, hbm, hbm, hbm, vmem],
        out_specs=hbm,
        scratch_shapes=[
            pltpu.VMEM((S, D), BF16),
            pltpu.VMEM((S, D), BF16),
            pltpu.VMEM((S, D), F32),
            pltpu.VMEM((L, D), F32),
            pltpu.VMEM((3, H * DH, D), BF16),
            pltpu.VMEM((H * DH, D), BF16),
            pltpu.VMEM((D // 2, 3 * H * DH), U32),
            pltpu.VMEM((H * DH // 2, D), U32),
            pltpu.VMEM((D, 3 * D), BF16),
            pltpu.VMEM((D, D), BF16),
            pltpu.VMEM((3 * D // 2, D), U32),
            pltpu.VMEM((D // 2, D), U32),
            pltpu.VMEM((NT_, 3 * D, 128), F32),
            pltpu.VMEM((3 * NT_, RB, 128), F32),
            pltpu.VMEM((3 * NT_, HALO + RB, 128), F32),
            pltpu.VMEM((RB, D), F32),
            pltpu.VMEM((RB, D), F32),
            pltpu.VMEM((2, RB // 2, D), U32),
            pltpu.SemaphoreType.DMA((NP,)),
            pltpu.SemaphoreType.DMA((4 + cfg.get('nwo', 1),)),
            pltpu.SemaphoreType.DMA((1,)),
        ],
        compiler_params=pltpu.CompilerParams(vmem_limit_bytes=120 * 1024 * 1024,
                                             disable_bounds_checks=True),
    )(A_x.reshape(S, D), A_mem0.reshape(M, D), wt(A_Wq), wt(A_Wk), wt(A_Wv),
      A_Wo.reshape(H * DH, D), B_wqkv, B_wo, gate_w)
    return out.reshape(1, S, D)


@functools.partial(jax.jit, static_argnames=("A_seg_len",))
def pallas_gated_mix__memory_aug_recurrent_mem_tr__sliding_local_dilated__prompt_kernel(
    A_x: jax.Array,
    A_mem0: jax.Array,
    A_Wq: jax.Array,
    A_Wk: jax.Array,
    A_Wv: jax.Array,
    A_Wo: jax.Array,
    A_seg_len: int,
    B_x: jax.Array,
    B_wqkv: jax.Array,
    B_wo: jax.Array,
    gate_w: jax.Array,
):
    del B_x
    assert A_seg_len == SEG
    assert A_x.shape == (1, S, D) and A_Wq.shape == (D, H, DH) and A_mem0.shape == (1, M, D)
    return _forward({}, A_x, A_mem0, A_Wq, A_Wk, A_Wv, A_Wo, B_wqkv, B_wo, gate_w)
```

```python
import functools

import jax
import jax.numpy as jnp
from jax.experimental import pallas as pl
from jax.experimental.pallas import tpu as pltpu

F32 = jnp.float32
BF16 = jnp.bfloat16
U32 = jnp.uint32

S = 2048
D = 640
H = 32
DH = 192
M = 8
SEG = 32
L = M + SEG
NSEG = S // SEG
NP = H // 2
PW = 2 * DH
MASK_VALUE = -1e9
LOG2E = 1.4426950408889634
HB = 32
DB = D // HB
WIN = 8
DIL = 2
RB = 128
XA0 = 256
XA1 = 768
NB = S // RB
HALO = 16
NT_ = D // 128


NN = (((1,), (0,)), ((), ()))
NT = (((1,), (1,)), ((), ()))


def _dot(a, b, dims=NN):
    return jax.lax.dot_general(a, b, dims, preferred_element_type=F32)


def _w(x):
    return pltpu.bitcast(x, BF16)


def _pack(x):
    return pltpu.bitcast(x, U32)


def _recip(den):
    r = pl.reciprocal(den, approx=True)
    return r * (2.0 - den * r)


def _blockdiag(t):
    lo = jax.lax.broadcasted_iota(jnp.int32, (L, 128), 1) < 64
    z = jnp.zeros((L, 128), F32)
    t0, t1, t2 = t[:, 0:128], t[:, 128:256], t[:, 256:384]
    top = jnp.concatenate([t0, jnp.where(lo, t1, 0.0), z], axis=1)
    bot = jnp.concatenate([z, jnp.where(lo, 0.0, t1), t2], axis=1)
    return jnp.concatenate([top, bot], axis=0).astype(BF16)


def _kernel(cfg, xa_hbm, mem_ref, wq_hbm, wk_hbm, wv_hbm, wo_hbm,
            wqkvb_hbm, wob_hbm, gate_ref,
            out_hbm,
            xa_v, out_v, b_v, h_ref,
            stage, wo_stage, w32, wo32,
            wqkvb_v, wob_v, wqkvb32, wob32, prep, fresh, cur, onew, ocur, x32,
            sem_qkv, sem_b, sem_in, sem_out):
    def qkv_copies(p):
        rows = pl.ds(pl.multiple_of(p * PW, 128), PW)
        return [pltpu.make_async_copy(src.at[rows, :], stage.at[i, rows, :], sem_qkv.at[p])
                for i, src in enumerate((wq_hbm, wk_hbm, wv_hbm))]

    nwo = cfg.get('nwo', 1)
    wo_rows = H * DH // nwo
    c_wo = [pltpu.make_async_copy(wo_hbm.at[i * wo_rows:(i + 1) * wo_rows, :],
                                  wo_stage.at[i * wo_rows:(i + 1) * wo_rows, :], sem_in.at[4 + i])
            for i in range(nwo)]
    c_wqkvb = [pltpu.make_async_copy(wqkvb_hbm.at[:, i * D:(i + 1) * D],
                                     wqkvb_v.at[:, i * D:(i + 1) * D], sem_b.at[i])
               for i in range(3)]
    c_wob = pltpu.make_async_copy(wob_hbm, wob_v, sem_in.at[1])
    c_xa0 = pltpu.make_async_copy(xa_hbm.at[0:XA0, :], xa_v.at[0:XA0, :], sem_in.at[2])
    c_xa1 = pltpu.make_async_copy(xa_hbm.at[XA0:XA1, :], xa_v.at[XA0:XA1, :], sem_in.at[3])
    c_xa2 = pltpu.make_async_copy(xa_hbm.at[XA1:S, :], xa_v.at[XA1:S, :], sem_b.at[3])
    c_xa0.start()
    for c in c_wqkvb:
        c.start()
    c_wob.start(priority=1)
    c_xa1.start(priority=1)

    def prep_wqkvb(part):
        for c in range(part * NT_, (part + 1) * NT_):
            t = wqkvb_v[:, c * 128:(c + 1) * 128].astype(F32).T
            for kt in range(NT_):
                prep[kt, c * 128:(c + 1) * 128, :] = t[:, kt * 128:(kt + 1) * 128]
        for d in range(DB):
            rows = jnp.concatenate(
                [prep[kt, pl.ds(part * D + d, HB, stride=DB), :] for kt in range(NT_)], axis=1)
            r0 = (part * D + d * HB) // 2
            wqkvb32[r0:r0 + HB // 2, :] = _pack(rows.astype(BF16))

    def prep_wob():
        for kt in range(NT_):
            prep[kt, 0:D, :] = wob_v[:, kt * 128:(kt + 1) * 128].astype(F32)
        for d in range(DB):
            rows = jnp.concatenate(
                [prep[kt, pl.ds(d, HB, stride=DB), :] for kt in range(NT_)], axis=1)
            wob32[d * (HB // 2):(d + 1) * (HB // 2), :] = _pack(rows.astype(BF16))

    def b_project(blk, first=False, part=None):
        xp = x32.at[1 if first else 0]
        if not part:
            xp[...] = _pack(xa_v[pl.ds(pl.multiple_of(blk * RB, RB), RB), :])
        tiles = range(3 * NT_) if part is None else range(part * NT_, (part + 1) * NT_)
        for j in tiles:
            x = _w(xp[...])
            y = _dot(x, _w(wqkvb32[j * 64:(j + 1) * 64, :]), NT)
            if first:
                cur[j, HALO:HALO + RB, :] = y
                if j >= NT_:
                    cur[j, 0:HALO, :] = jnp.zeros((HALO, 128), F32)
            else:
                fresh[j] = y

    def b_rotate():
        for j in range(NT_, 3 * NT_):
            cur[j, 0:HALO, :] = cur[j, RB:RB + HALO, :]
        for j in range(3 * NT_):
            cur[j, HALO:HALO + RB, :] = fresh[j]
        ocur[...] = onew[...]

    def b_attend_rows(base, n, row0):
        src = cur
        q = [src[j, HALO + base:HALO + base + n, :] for j in range(NT_)]
        row = jax.lax.broadcasted_iota(jnp.int32, (n, 128), 0) + (row0 + base)
        half = WIN // 2
        step = DIL * half
        logits = [None] * WIN
        for w in range(half):
            o = HALO + base - DIL * w - step
            lo = hi = None
            for j in range(NT_):
                k = src[NT_ + j, o:o + n + step, :]
                a, b = q[j] * k[step:], q[j] * k[:n]
                lo = a if lo is None else lo + a
                hi = b if hi is None else hi + b
            for ww, s in ((w, lo), (w + half, hi)):
                s = s + pltpu.roll(s, 64, 1)
                s = s + pltpu.roll(s, 32, 1)
                s = s * (DB ** -0.5 * LOG2E)
                if ww:
                    s = jnp.where(row >= DIL * ww, s, MASK_VALUE * LOG2E)
                logits[ww] = s
        m = logits[0]
        for w in range(1, WIN):
            m = jnp.maximum(m, logits[w])
        e = [jnp.exp2(l - m) for l in logits]
        den = e[0]
        for w in range(1, WIN):
            den = den + e[w]
        r = _recip(den)
        outs = []
        for j in range(NT_):
            acc = None
            for w in range(half):
                o = HALO + base - DIL * w - step
                v = src[2 * NT_ + j, o:o + n + step, :]
                t = e[w] * v[step:] + e[w + half] * v[:n]
                acc = t if acc is None else acc + t
            outs.append(acc * r)
        return jnp.concatenate(outs, axis=1)

    def b_attend(blk, between=()):
        sub = cfg.get('sub', 64)
        between = list(between)
        for base in range(0, RB, sub):
            if between:
                between.pop(0)()
            onew[base:base + sub, :] = b_attend_rows(base, sub, blk * RB)
        for f in between:
            f()

    def b_output(blk, src):
        b_v[pl.ds(pl.multiple_of(blk * RB, RB), RB), :] = _dot(src[...], _w(wob32[...]))

    def qkv_weight(p, i):
        if cfg.get('nodma'):
            return
        rows = pl.ds(pl.multiple_of(p * PW, 128), PW)
        col = pl.multiple_of(p * 3 * PW, 128)
        w32[:, pl.ds(col + i * PW, PW)] = _pack(stage[i, rows, :].astype(F32).T.astype(BF16))

    def qkv_weights(p):
        for i in range(3):
            qkv_weight(p, i)

    def wait_qkv(p):
        if cfg.get('nodma'):
            return
        for c in qkv_copies(p):
            c.wait()

    c_xa0.wait()
    c_wqkvb[0].wait()
    n_early = cfg.get('x2_pos', 4)
    for p in range(n_early):
        for c in qkv_copies(p):
            c.start(priority=1)
    prep_wqkvb(0)
    c_wqkvb[1].wait()
    c_xa2.start(priority=1)
    prep_wqkvb(1)
    b_project(0, first=True, part=0)
    c_wqkvb[2].wait()
    for p in range(n_early, NP):
        for c in qkv_copies(p):
            c.start(priority=1)
    prep_wqkvb(2)
    b_project(0, first=True, part=1)
    c_wob.wait()
    b_project(0, first=True, part=2)
    if not cfg.get('nodma') and not cfg.get('nowo'):
        for c in c_wo:
            c.start(priority=1)
    if cfg.get('wob_pos', 2) == 0:
        prep_wob()
    b_project(1)
    if cfg.get('wob_pos', 2) == 1:
        prep_wob()
    b_attend(0)
    if cfg.get('wob_pos', 2) == 2:
        prep_wob()
    b_rotate()
    c_xa1.wait()

    def p1_step(k):
        for c in cfg.get('order', 'poatr'):
            if c == 'p':
                b_project(k + 1)
            elif c == 'o':
                b_output(k - 1, ocur)
            elif c == 'a':
                b_attend(k)
            elif c == 't':
                qkv_weights(k - 1)
            elif c == 'r':
                b_rotate()

    unroll = cfg.get('unroll', 1)

    def p1_body(i, carry):
        k0 = 1 + unroll * i

        @pl.when(k0 == XA1 // RB - 1)
        def _():
            c_xa2.wait()

        for u in range(unroll):
            wait_qkv(k0 + u - 1)
        for u in range(unroll):
            p1_step(k0 + u)
        return carry

    jax.lax.fori_loop(0, (NB - 2) // unroll, p1_body, 0)
    wait_qkv(NB - 2)
    wait_qkv(NB - 1)
    b_output(NB - 2, ocur)
    if cfg.get('batt_t', 0) < 0:
        b_attend(NB - 1)
    qkv_weights(NB - 2)
    qkv_weights(NB - 1)

    if cfg.get('stop_after_p1'):
        if not cfg.get('nowo'):
            for c in c_wo:
                c.wait()
        return
    h_ref[0:M, :] = mem_ref[...].astype(F32)
    gate = gate_ref[...].astype(F32).reshape(1, D)
    lag_b, lag_e, lag_f = cfg.get('lags', (1, 4, 8))

    def segment(s, carry, first=False):
        off = s * SEG if first else pl.multiple_of(s * SEG, SEG)
        x = xa_v[pl.ds(off, SEG), :].astype(F32)
        h_ref[M:L, :] = x
        r = jax.lax.broadcasted_iota(jnp.int32, (L, 2 * L), 0)
        c = jax.lax.broadcasted_iota(jnp.int32, (L, 2 * L), 1)
        isb = c >= L
        key = jnp.where(isb, c - L, c)
        allowed = (r < M) | (r >= key)
        st = [dict() for _ in range(NP)]
        acc = [None]

        def project(p):
            h = h_ref[...]
            b = p * 3 * PW
            st[p]['q'] = _dot(h, _w(w32[:, b:b + PW]))
            st[p]['kb'] = _blockdiag(_dot(h, _w(w32[:, b + PW:b + 2 * PW])))
            st[p]['vb'] = _blockdiag(_dot(h, _w(w32[:, b + 2 * PW:b + 3 * PW])))

        def softmax(p):
            sc = _dot(st[p].pop('q'), st[p].pop('kb'), NT)
            t = jnp.where(allowed, sc * (DH ** -0.5 * LOG2E), MASK_VALUE * LOG2E)
            ma = jnp.max(jnp.where(isb, -jnp.inf, t), axis=1, keepdims=True)
            mb = jnp.max(jnp.where(isb, t, -jnp.inf), axis=1, keepdims=True)
            e = jnp.exp2(t - jnp.where(isb, mb, ma))
            sa = jnp.sum(jnp.where(isb, 0.0, e), axis=1, keepdims=True)
            sb = jnp.sum(jnp.where(isb, e, 0.0), axis=1, keepdims=True)
            st[p]['p'] = e * _recip(jnp.where(isb, sb, sa))

        def values(p):
            st[p]['o'] = _dot(st[p].pop('p'), st[p].pop('vb'))

        def output(p):
            if first:
                w = wo_stage[p * PW:(p + 1) * PW, :]
                wo32[p * (PW // 2):(p + 1) * (PW // 2), :] = _pack(w)
            else:
                w = _w(wo32[p * (PW // 2):(p + 1) * (PW // 2), :])
            y = _dot(st[p].pop('o'), w)
            acc[0] = y if acc[0] is None else acc[0] + y

        nsteps = NP + (lag_e + 1 if first else lag_f)
        wo_t = cfg.get('wo_t', (nsteps - 1,))
        for t in range(nsteps):
            if t < NP:
                project(t)
            if first and t == cfg.get('batt_t', 0):
                b_attend(NB - 1)
            if first and t == cfg.get('bout_t', 16):
                b_output(NB - 1, onew)
            if 0 <= t - lag_b < NP:
                softmax(t - lag_b)
            if 0 <= t - lag_e < NP:
                values(t - lag_e)
            if not first and 0 <= t - lag_f < NP:
                output(t - lag_f)
            if first:
                for i, tw in enumerate(wo_t):
                    if t == tw and not cfg.get('nodma'):
                        c_wo[i].wait()
                    if t >= tw:
                        lo, hi = i * NP // nwo, (i + 1) * NP // nwo
                        per = -(-(hi - lo) // (nsteps - tw)) if tw < nsteps else hi - lo
                        for p in range(lo + (t - tw) * per, min(hi, lo + (t - tw + 1) * per)):
                            output(p)
        a = acc[0]
        h_ref[0:M, :] = a[0:M]
        z = jnp.sum(x * gate, axis=1, keepdims=True)
        g = 1.0 / (1.0 + jnp.exp(-z))
        y = g * a[M:L] + (1.0 - g) * b_v[pl.ds(off, SEG), :]
        out_v[pl.ds(off, SEG), :] = y.astype(out_v.dtype)
        pltpu.make_async_copy(out_v.at[pl.ds(off, SEG), :], out_hbm.at[pl.ds(off, SEG), :],
                              sem_out.at[0]).start()
        return carry

    nseg = cfg.get('nseg', NSEG)
    if cfg.get('peel', True):
        segment(0, 0, first=True)
        start = 1
    else:
        b_attend(NB - 1)
        b_output(NB - 1, onew)
        for c in c_wo:
            c.wait()
        for p in range(NP):
            wo32[p * (PW // 2):(p + 1) * (PW // 2), :] = _pack(wo_stage[p * PW:(p + 1) * PW, :])
        start = 0
    if nseg > start:
        jax.lax.fori_loop(start, nseg, segment, 0)
    n_out = max(nseg, start)
    if n_out:
        pltpu.make_async_copy(out_v.at[0:n_out * SEG, :], out_hbm.at[0:n_out * SEG, :],
                              sem_out.at[0]).wait()


def _forward(cfg, A_x, A_mem0, A_Wq, A_Wk, A_Wv, A_Wo, B_wqkv, B_wo, gate_w):
    def wt(w):
        return jnp.transpose(w, (1, 2, 0)).reshape(H * DH, D)

    hbm = pl.BlockSpec(memory_space=pl.ANY)
    vmem = pl.BlockSpec(memory_space=pltpu.VMEM)
    out = pl.pallas_call(
        functools.partial(_kernel, cfg),
        out_shape=jax.ShapeDtypeStruct((S, D), BF16),
        in_specs=[hbm, vmem, hbm, hbm, hbm, hbm, hbm, hbm, vmem],
        out_specs=hbm,
        scratch_shapes=[
            pltpu.VMEM((S, D), BF16),
            pltpu.VMEM((S, D), BF16),
            pltpu.VMEM((S, D), F32),
            pltpu.VMEM((L, D), F32),
            pltpu.VMEM((3, H * DH, D), BF16),
            pltpu.VMEM((H * DH, D), BF16),
            pltpu.VMEM((D // 2, 3 * H * DH), U32),
            pltpu.VMEM((H * DH // 2, D), U32),
            pltpu.VMEM((D, 3 * D), BF16),
            pltpu.VMEM((D, D), BF16),
            pltpu.VMEM((3 * D // 2, D), U32),
            pltpu.VMEM((D // 2, D), U32),
            pltpu.VMEM((NT_, 3 * D, 128), F32),
            pltpu.VMEM((3 * NT_, RB, 128), F32),
            pltpu.VMEM((3 * NT_, HALO + RB, 128), F32),
            pltpu.VMEM((RB, D), F32),
            pltpu.VMEM((RB, D), F32),
            pltpu.VMEM((2, RB // 2, D), U32),
            pltpu.SemaphoreType.DMA((NP,)),
            pltpu.SemaphoreType.DMA((4,)),
            pltpu.SemaphoreType.DMA((4 + cfg.get('nwo', 1),)),
            pltpu.SemaphoreType.DMA((1,)),
        ],
        compiler_params=pltpu.CompilerParams(vmem_limit_bytes=120 * 1024 * 1024,
                                             disable_bounds_checks=True),
    )(A_x.reshape(S, D), A_mem0.reshape(M, D), wt(A_Wq), wt(A_Wk), wt(A_Wv),
      A_Wo.reshape(H * DH, D), B_wqkv, B_wo, gate_w)
    return out.reshape(1, S, D)


@functools.partial(jax.jit, static_argnames=("A_seg_len",))
def pallas_gated_mix__memory_aug_recurrent_mem_tr__sliding_local_dilated__prompt_kernel(
    A_x: jax.Array,
    A_mem0: jax.Array,
    A_Wq: jax.Array,
    A_Wk: jax.Array,
    A_Wv: jax.Array,
    A_Wo: jax.Array,
    A_seg_len: int,
    B_x: jax.Array,
    B_wqkv: jax.Array,
    B_wo: jax.Array,
    gate_w: jax.Array,
):
    del B_x
    assert A_seg_len == SEG
    assert A_x.shape == (1, S, D) and A_Wq.shape == (D, H, DH) and A_mem0.shape == (1, M, D)
    return _forward({}, A_x, A_mem0, A_Wq, A_Wk, A_Wv, A_Wo, B_wqkv, B_wo, gate_w)
```

```python
import functools

import jax
import jax.numpy as jnp
from jax.experimental import pallas as pl
from jax.experimental.pallas import tpu as pltpu

F32 = jnp.float32
BF16 = jnp.bfloat16
U32 = jnp.uint32

S = 2048
D = 640
H = 32
DH = 192
M = 8
SEG = 32
L = M + SEG
NSEG = S // SEG
NP = H // 2
PW = 2 * DH
MASK_VALUE = -1e9
LOG2E = 1.4426950408889634
HB = 32
DB = D // HB
WIN = 8
DIL = 2
RB = 128
XA0 = 256
XA1 = 768
NB = S // RB
HALO = 16
NT_ = D // 128


NN = (((1,), (0,)), ((), ()))
NT = (((1,), (1,)), ((), ()))


def _dot(a, b, dims=NN):
    return jax.lax.dot_general(a, b, dims, preferred_element_type=F32)


def _w(x):
    return pltpu.bitcast(x, BF16)


def _pack(x):
    return pltpu.bitcast(x, U32)


def _recip(den):
    r = pl.reciprocal(den, approx=True)
    return r * (2.0 - den * r)


def _blockdiag(t):
    lo = jax.lax.broadcasted_iota(jnp.int32, (L, 128), 1) < 64
    z = jnp.zeros((L, 128), F32)
    t0, t1, t2 = t[:, 0:128], t[:, 128:256], t[:, 256:384]
    top = jnp.concatenate([t0, jnp.where(lo, t1, 0.0), z], axis=1)
    bot = jnp.concatenate([z, jnp.where(lo, 0.0, t1), t2], axis=1)
    return jnp.concatenate([top, bot], axis=0).astype(BF16)


def _kernel(cfg, xa_hbm, mem_ref, wq_hbm, wk_hbm, wv_hbm, wo_hbm,
            wqkvb_hbm, wob_hbm, gate_ref,
            out_hbm,
            xa_v, out_v, b_v, h_ref,
            stage, wo_stage, w32, wo32,
            wqkvb_v, wob_v, wqkvb32, wob32, prep, fresh, cur, onew, ocur, x32,
            sem_qkv, sem_b, sem_in, sem_out):
    def qkv_copies(p):
        rows = pl.ds(pl.multiple_of(p * PW, 128), PW)
        return [pltpu.make_async_copy(src.at[rows, :], stage.at[i, rows, :], sem_qkv.at[p])
                for i, src in enumerate((wq_hbm, wk_hbm, wv_hbm))]

    nwo = cfg.get('nwo', 1)
    wo_rows = H * DH // nwo
    c_wo = [pltpu.make_async_copy(wo_hbm.at[i * wo_rows:(i + 1) * wo_rows, :],
                                  wo_stage.at[i * wo_rows:(i + 1) * wo_rows, :], sem_in.at[4 + i])
            for i in range(nwo)]
    c_wqkvb = [pltpu.make_async_copy(wqkvb_hbm.at[:, i * D:(i + 1) * D],
                                     wqkvb_v.at[:, i * D:(i + 1) * D], sem_b.at[i])
               for i in range(3)]
    c_wob = pltpu.make_async_copy(wob_hbm, wob_v, sem_in.at[1])
    c_xa0 = pltpu.make_async_copy(xa_hbm.at[0:XA0, :], xa_v.at[0:XA0, :], sem_in.at[2])
    c_xa1 = pltpu.make_async_copy(xa_hbm.at[XA0:XA1, :], xa_v.at[XA0:XA1, :], sem_in.at[3])
    c_xa2 = pltpu.make_async_copy(xa_hbm.at[XA1:S, :], xa_v.at[XA1:S, :], sem_b.at[3])
    c_xa0.start()
    for c in c_wqkvb:
        c.start()
    c_wob.start(priority=1)
    c_xa1.start(priority=1)

    def prep_wqkvb(part):
        for c in range(part * NT_, (part + 1) * NT_):
            t = wqkvb_v[:, c * 128:(c + 1) * 128].astype(F32).T
            for kt in range(NT_):
                prep[kt, c * 128:(c + 1) * 128, :] = t[:, kt * 128:(kt + 1) * 128]
        for d in range(DB):
            rows = jnp.concatenate(
                [prep[kt, pl.ds(part * D + d, HB, stride=DB), :] for kt in range(NT_)], axis=1)
            r0 = (part * D + d * HB) // 2
            wqkvb32[r0:r0 + HB // 2, :] = _pack(rows.astype(BF16))

    def prep_wob():
        for kt in range(NT_):
            prep[kt, 0:D, :] = wob_v[:, kt * 128:(kt + 1) * 128].astype(F32)
        for d in range(DB):
            rows = jnp.concatenate(
                [prep[kt, pl.ds(d, HB, stride=DB), :] for kt in range(NT_)], axis=1)
            wob32[d * (HB // 2):(d + 1) * (HB // 2), :] = _pack(rows.astype(BF16))

    def b_project(blk, first=False, part=None):
        xp = x32.at[1 if first else 0]
        if not part:
            xp[...] = _pack(xa_v[pl.ds(pl.multiple_of(blk * RB, RB), RB), :])
        tiles = range(3 * NT_) if part is None else range(part * NT_, (part + 1) * NT_)
        for j in tiles:
            x = _w(xp[...])
            y = _dot(x, _w(wqkvb32[j * 64:(j + 1) * 64, :]), NT)
            if first:
                cur[j, HALO:HALO + RB, :] = y
                if j >= NT_:
                    cur[j, 0:HALO, :] = jnp.zeros((HALO, 128), F32)
            else:
                fresh[j] = y

    def b_rotate():
        for j in range(NT_, 3 * NT_):
            cur[j, 0:HALO, :] = cur[j, RB:RB + HALO, :]
        for j in range(3 * NT_):
            cur[j, HALO:HALO + RB, :] = fresh[j]
        ocur[...] = onew[...]

    def b_attend_rows(base, n, row0):
        src = cur
        q = [src[j, HALO + base:HALO + base + n, :] for j in range(NT_)]
        row = jax.lax.broadcasted_iota(jnp.int32, (n, 128), 0) + (row0 + base)
        half = WIN // 2
        step = DIL * half
        logits = [None] * WIN
        for w in range(half):
            o = HALO + base - DIL * w - step
            lo = hi = None
            for j in range(NT_):
                k = src[NT_ + j, o:o + n + step, :]
                a, b = q[j] * k[step:], q[j] * k[:n]
                lo = a if lo is None else lo + a
                hi = b if hi is None else hi + b
            for ww, s in ((w, lo), (w + half, hi)):
                s = s + pltpu.roll(s, 64, 1)
                s = s + pltpu.roll(s, 32, 1)
                s = s * (DB ** -0.5 * LOG2E)
                if ww:
                    s = jnp.where(row >= DIL * ww, s, MASK_VALUE * LOG2E)
                logits[ww] = s
        m = logits[0]
        for w in range(1, WIN):
            m = jnp.maximum(m, logits[w])
        e = [jnp.exp2(l - m) for l in logits]
        den = e[0]
        for w in range(1, WIN):
            den = den + e[w]
        r = _recip(den)
        outs = []
        for j in range(NT_):
            acc = None
            for w in range(half):
                o = HALO + base - DIL * w - step
                v = src[2 * NT_ + j, o:o + n + step, :]
                t = e[w] * v[step:] + e[w + half] * v[:n]
                acc = t if acc is None else acc + t
            outs.append(acc * r)
        return jnp.concatenate(outs, axis=1)

    def b_attend(blk, between=()):
        sub = cfg.get('sub', 64)
        between = list(between)
        for base in range(0, RB, sub):
            if between:
                between.pop(0)()
            onew[base:base + sub, :] = b_attend_rows(base, sub, blk * RB)
        for f in between:
            f()

    def b_output(blk, src):
        b_v[pl.ds(pl.multiple_of(blk * RB, RB), RB), :] = _dot(src[...], _w(wob32[...]))

    def qkv_weight(p, i):
        if cfg.get('nodma'):
            return
        rows = pl.ds(pl.multiple_of(p * PW, 128), PW)
        col = pl.multiple_of(p * 3 * PW, 128)
        w32[:, pl.ds(col + i * PW, PW)] = _pack(stage[i, rows, :].astype(F32).T.astype(BF16))

    def qkv_weights(p):
        for i in range(3):
            qkv_weight(p, i)

    def wait_qkv(p):
        if cfg.get('nodma'):
            return
        for c in qkv_copies(p):
            c.wait()

    c_xa0.wait()
    c_wqkvb[0].wait()
    n_early = cfg.get('x2_pos', 4)
    for p in range(n_early):
        for c in qkv_copies(p):
            c.start(priority=1)
    prep_wqkvb(0)
    c_wqkvb[1].wait()
    c_xa2.start(priority=1)
    prep_wqkvb(1)
    b_project(0, first=True, part=0)
    c_wqkvb[2].wait()
    for p in range(n_early, NP):
        for c in qkv_copies(p):
            c.start(priority=1)
    prep_wqkvb(2)
    b_project(0, first=True, part=1)
    c_wob.wait()
    b_project(0, first=True, part=2)
    if not cfg.get('nodma') and not cfg.get('nowo'):
        for c in c_wo:
            c.start(priority=1)
    if cfg.get('wob_pos', 2) == 0:
        prep_wob()
    b_project(1)
    if cfg.get('wob_pos', 2) == 1:
        prep_wob()
    b_attend(0)
    if cfg.get('wob_pos', 2) == 2:
        prep_wob()
    b_rotate()
    c_xa1.wait()

    def p1_step(k):
        for c in cfg.get('order', 'poatr'):
            if c == 'p':
                b_project(k + 1)
            elif c == 'o':
                b_output(k - 1, ocur)
            elif c == 'a':
                b_attend(k)
            elif c == 't':
                qkv_weights(k - 1)
            elif c == 'r':
                b_rotate()

    unroll = cfg.get('unroll', 1)

    def p1_body(i, carry):
        k0 = 1 + unroll * i

        @pl.when(k0 == XA1 // RB - 1)
        def _():
            c_xa2.wait()

        for u in range(unroll):
            wait_qkv(k0 + u - 1)
        for u in range(unroll):
            p1_step(k0 + u)
        return carry

    jax.lax.fori_loop(0, (NB - 2) // unroll, p1_body, 0)
    wait_qkv(NB - 2)
    wait_qkv(NB - 1)
    b_output(NB - 2, ocur)
    if cfg.get('batt_t', 0) < 0:
        b_attend(NB - 1)
    qkv_weights(NB - 2)
    qkv_weights(NB - 1)

    if cfg.get('stop_after_p1'):
        if not cfg.get('nowo'):
            for c in c_wo:
                c.wait()
        return
    mem_last = cfg.get('mem_last', True)
    out_mem_first = cfg.get('out_mem_first', True)
    X0, M0 = (0, SEG) if mem_last else (M, 0)
    h_ref[M0:M0 + M, :] = mem_ref[...].astype(F32)
    gate = gate_ref[...].astype(F32).reshape(1, D)
    lag_b, lag_e, lag_f = cfg.get('lags', (1, 4, 8))

    def segment(s, carry, first=False, static=False):
        off = s * SEG if first or static else pl.multiple_of(s * SEG, SEG)
        x = xa_v[pl.ds(off, SEG), :].astype(F32)
        h_ref[X0:X0 + SEG, :] = x
        r = jax.lax.broadcasted_iota(jnp.int32, (L, 2 * L), 0)
        c = jax.lax.broadcasted_iota(jnp.int32, (L, 2 * L), 1)
        isb = c >= L
        key = jnp.where(isb, c - L, c)
        if mem_last:
            allowed = (r >= SEG) | (key >= SEG) | (r >= key)
        else:
            allowed = (r < M) | (r >= key)
        st = [dict() for _ in range(NP)]
        acc = [None]

        def project(p):
            h = h_ref[...]
            b = p * 3 * PW
            st[p]['q'] = _dot(h, _w(w32[:, b:b + PW]))
            st[p]['kb'] = _blockdiag(_dot(h, _w(w32[:, b + PW:b + 2 * PW])))
            st[p]['vb'] = _blockdiag(_dot(h, _w(w32[:, b + 2 * PW:b + 3 * PW])))

        def softmax(p):
            sc = _dot(st[p].pop('q'), st[p].pop('kb'), NT)
            t = jnp.where(allowed, sc * (DH ** -0.5 * LOG2E), MASK_VALUE * LOG2E)
            ma = jnp.max(jnp.where(isb, -jnp.inf, t), axis=1, keepdims=True)
            mb = jnp.max(jnp.where(isb, t, -jnp.inf), axis=1, keepdims=True)
            e = jnp.exp2(t - jnp.where(isb, mb, ma))
            sa = jnp.sum(jnp.where(isb, 0.0, e), axis=1, keepdims=True)
            sb = jnp.sum(jnp.where(isb, e, 0.0), axis=1, keepdims=True)
            st[p]['p'] = e * _recip(jnp.where(isb, sb, sa))

        def values(p):
            st[p]['o'] = _dot(st[p].pop('p'), st[p].pop('vb'))

        def output(p):
            if first:
                w = wo_stage[p * PW:(p + 1) * PW, :]
                wo32[p * (PW // 2):(p + 1) * (PW // 2), :] = _pack(w)
            else:
                w = _w(wo32[p * (PW // 2):(p + 1) * (PW // 2), :])
            o = st[p].pop('o')
            if mem_last and out_mem_first:
                o = jnp.concatenate([o[SEG:L], o[0:SEG]], axis=0)
            y = _dot(o, w)
            acc[0] = y if acc[0] is None else acc[0] + y

        nsteps = NP + (lag_e + 1 if first else lag_f)
        wo_t = cfg.get('wo_t', (nsteps - 1,))
        for t in range(nsteps):
            if t < NP:
                project(t)
            if first and t == cfg.get('batt_t', 0):
                b_attend(NB - 1)
            if first and t == cfg.get('bout_t', 16):
                b_output(NB - 1, onew)
            if 0 <= t - lag_b < NP:
                softmax(t - lag_b)
            if 0 <= t - lag_e < NP:
                values(t - lag_e)
            if not first and 0 <= t - lag_f < NP:
                output(t - lag_f)
            if first:
                for i, tw in enumerate(wo_t):
                    if t == tw and not cfg.get('nodma'):
                        c_wo[i].wait()
                    if t >= tw:
                        lo, hi = i * NP // nwo, (i + 1) * NP // nwo
                        per = -(-(hi - lo) // (nsteps - tw)) if tw < nsteps else hi - lo
                        for p in range(lo + (t - tw) * per, min(hi, lo + (t - tw + 1) * per)):
                            output(p)
        a = acc[0]
        if mem_last and not out_mem_first:
            a_mem, a_x = a[SEG:L], a[0:SEG]
        else:
            a_mem, a_x = a[0:M], a[M:L]
        h_ref[M0:M0 + M, :] = a_mem
        z = jnp.sum(x * gate, axis=1, keepdims=True)
        g = 1.0 / (1.0 + jnp.exp(-z))
        y = g * a_x + (1.0 - g) * b_v[pl.ds(off, SEG), :]
        out_v[pl.ds(off, SEG), :] = y.astype(out_v.dtype)
        pltpu.make_async_copy(out_v.at[pl.ds(off, SEG), :], out_hbm.at[pl.ds(off, SEG), :],
                              sem_out.at[0]).start()
        return carry

    nseg = cfg.get('nseg', NSEG)
    if cfg.get('peel', True):
        segment(0, 0, first=True)
        start = 1
    else:
        b_attend(NB - 1)
        b_output(NB - 1, onew)
        for c in c_wo:
            c.wait()
        for p in range(NP):
            wo32[p * (PW // 2):(p + 1) * (PW // 2), :] = _pack(wo_stage[p * PW:(p + 1) * PW, :])
        start = 0
    su = cfg.get('seg_unroll', 3)
    if su > 1:
        while (nseg - start) % su:
            segment(start, 0, static=True)
            start += 1

        def segments(i, carry):
            for u in range(su):
                segment(start + i * su + u, carry)
            return carry
        jax.lax.fori_loop(0, (nseg - start) // su, segments, 0)
    elif nseg > start:
        jax.lax.fori_loop(start, nseg, segment, 0)
    n_out = max(nseg, start)
    if n_out:
        pltpu.make_async_copy(out_v.at[0:n_out * SEG, :], out_hbm.at[0:n_out * SEG, :],
                              sem_out.at[0]).wait()


def _forward(cfg, A_x, A_mem0, A_Wq, A_Wk, A_Wv, A_Wo, B_wqkv, B_wo, gate_w):
    def wt(w):
        return jnp.transpose(w, (1, 2, 0)).reshape(H * DH, D)

    hbm = pl.BlockSpec(memory_space=pl.ANY)
    vmem = pl.BlockSpec(memory_space=pltpu.VMEM)
    out = pl.pallas_call(
        functools.partial(_kernel, cfg),
        out_shape=jax.ShapeDtypeStruct((S, D), BF16),
        in_specs=[hbm, vmem, hbm, hbm, hbm, hbm, hbm, hbm, vmem],
        out_specs=hbm,
        scratch_shapes=[
            pltpu.VMEM((S, D), BF16),
            pltpu.VMEM((S, D), BF16),
            pltpu.VMEM((S, D), F32),
            pltpu.VMEM((L, D), F32),
            pltpu.VMEM((3, H * DH, D), BF16),
            pltpu.VMEM((H * DH, D), BF16),
            pltpu.VMEM((D // 2, 3 * H * DH), U32),
            pltpu.VMEM((H * DH // 2, D), U32),
            pltpu.VMEM((D, 3 * D), BF16),
            pltpu.VMEM((D, D), BF16),
            pltpu.VMEM((3 * D // 2, D), U32),
            pltpu.VMEM((D // 2, D), U32),
            pltpu.VMEM((NT_, 3 * D, 128), F32),
            pltpu.VMEM((3 * NT_, RB, 128), F32),
            pltpu.VMEM((3 * NT_, HALO + RB, 128), F32),
            pltpu.VMEM((RB, D), F32),
            pltpu.VMEM((RB, D), F32),
            pltpu.VMEM((2, RB // 2, D), U32),
            pltpu.SemaphoreType.DMA((NP,)),
            pltpu.SemaphoreType.DMA((4,)),
            pltpu.SemaphoreType.DMA((4 + cfg.get('nwo', 1),)),
            pltpu.SemaphoreType.DMA((1,)),
        ],
        compiler_params=pltpu.CompilerParams(vmem_limit_bytes=120 * 1024 * 1024,
                                             disable_bounds_checks=True),
    )(A_x.reshape(S, D), A_mem0.reshape(M, D), wt(A_Wq), wt(A_Wk), wt(A_Wv),
      A_Wo.reshape(H * DH, D), B_wqkv, B_wo, gate_w)
    return out.reshape(1, S, D)


@functools.partial(jax.jit, static_argnames=("A_seg_len",))
def pallas_gated_mix__memory_aug_recurrent_mem_tr__sliding_local_dilated__prompt_kernel(
    A_x: jax.Array,
    A_mem0: jax.Array,
    A_Wq: jax.Array,
    A_Wk: jax.Array,
    A_Wv: jax.Array,
    A_Wo: jax.Array,
    A_seg_len: int,
    B_x: jax.Array,
    B_wqkv: jax.Array,
    B_wo: jax.Array,
    gate_w: jax.Array,
):
    del B_x
    assert A_seg_len == SEG
    assert A_x.shape == (1, S, D) and A_Wq.shape == (D, H, DH) and A_mem0.shape == (1, M, D)
    return _forward({}, A_x, A_mem0, A_Wq, A_Wk, A_Wv, A_Wo, B_wqkv, B_wo, gate_w)
```

```python
import functools

import jax
import jax.numpy as jnp
from jax.experimental import pallas as pl
from jax.experimental.pallas import tpu as pltpu

F32 = jnp.float32
BF16 = jnp.bfloat16
U32 = jnp.uint32

S = 2048
D = 640
H = 32
DH = 192
M = 8
SEG = 32
L = M + SEG
NSEG = S // SEG
NP = H // 2
PW = 2 * DH
MASK_VALUE = -1e9
LOG2E = 1.4426950408889634
HB = 32
DB = D // HB
WIN = 8
DIL = 2
RB = 128
XA0 = 256
XA1 = 768
NB = S // RB
HALO = 16
NT_ = D // 128


NN = (((1,), (0,)), ((), ()))
NT = (((1,), (1,)), ((), ()))


def _dot(a, b, dims=NN):
    return jax.lax.dot_general(a, b, dims, preferred_element_type=F32)


def _w(x):
    return pltpu.bitcast(x, BF16)


def _pack(x):
    return pltpu.bitcast(x, U32)


def _recip(den):
    r = pl.reciprocal(den, approx=True)
    return r * (2.0 - den * r)


def _blockdiag(t):
    lo = jax.lax.broadcasted_iota(jnp.int32, (L, 128), 1) < 64
    z = jnp.zeros((L, 128), F32)
    t0, t1, t2 = t[:, 0:128], t[:, 128:256], t[:, 256:384]
    top = jnp.concatenate([t0, jnp.where(lo, t1, 0.0), z], axis=1)
    bot = jnp.concatenate([z, jnp.where(lo, 0.0, t1), t2], axis=1)
    return jnp.concatenate([top, bot], axis=0).astype(BF16)


def _kernel(cfg, xa_hbm, mem_ref, wq_hbm, wk_hbm, wv_hbm, wo_hbm,
            wqkvb_hbm, wob_hbm, gate_ref,
            out_hbm,
            xa_v, out_v, b_v, h_ref,
            stage, wo_stage, w32, wo32,
            wqkvb_v, wob_v, wqkvb32, wob32, prep, fresh, cur, onew, ocur, x32,
            sem_qkv, sem_b, sem_in, sem_out):
    def qkv_copies(p):
        rows = pl.ds(pl.multiple_of(p * PW, 128), PW)
        return [pltpu.make_async_copy(src.at[rows, :], stage.at[i, rows, :], sem_qkv.at[p])
                for i, src in enumerate((wq_hbm, wk_hbm, wv_hbm))]

    nwo = cfg.get('nwo', 1)
    wo_rows = H * DH // nwo
    c_wo = [pltpu.make_async_copy(wo_hbm.at[i * wo_rows:(i + 1) * wo_rows, :],
                                  wo_stage.at[i * wo_rows:(i + 1) * wo_rows, :], sem_in.at[4 + i])
            for i in range(nwo)]
    c_wqkvb = [pltpu.make_async_copy(wqkvb_hbm.at[:, i * D:(i + 1) * D],
                                     wqkvb_v.at[:, i * D:(i + 1) * D], sem_b.at[i])
               for i in range(3)]
    c_wob = pltpu.make_async_copy(wob_hbm, wob_v, sem_in.at[1])
    c_xa0 = pltpu.make_async_copy(xa_hbm.at[0:XA0, :], xa_v.at[0:XA0, :], sem_in.at[2])
    c_xa1 = pltpu.make_async_copy(xa_hbm.at[XA0:XA1, :], xa_v.at[XA0:XA1, :], sem_in.at[3])
    c_xa2 = pltpu.make_async_copy(xa_hbm.at[XA1:S, :], xa_v.at[XA1:S, :], sem_b.at[3])
    c_xa0.start()
    for c in c_wqkvb:
        c.start()
    c_wob.start(priority=1)
    c_xa1.start(priority=1)

    def prep_wqkvb(part):
        for c in range(part * NT_, (part + 1) * NT_):
            t = wqkvb_v[:, c * 128:(c + 1) * 128].astype(F32).T
            for kt in range(NT_):
                prep[kt, c * 128:(c + 1) * 128, :] = t[:, kt * 128:(kt + 1) * 128]
        for d in range(DB):
            rows = jnp.concatenate(
                [prep[kt, pl.ds(part * D + d, HB, stride=DB), :] for kt in range(NT_)], axis=1)
            r0 = (part * D + d * HB) // 2
            wqkvb32[r0:r0 + HB // 2, :] = _pack(rows.astype(BF16))

    def prep_wob():
        for kt in range(NT_):
            prep[kt, 0:D, :] = wob_v[:, kt * 128:(kt + 1) * 128].astype(F32)
        for d in range(DB):
            rows = jnp.concatenate(
                [prep[kt, pl.ds(d, HB, stride=DB), :] for kt in range(NT_)], axis=1)
            wob32[d * (HB // 2):(d + 1) * (HB // 2), :] = _pack(rows.astype(BF16))

    def b_project(blk, first=False, part=None):
        xp = x32.at[1 if first else 0]
        if not part:
            xp[...] = _pack(xa_v[pl.ds(pl.multiple_of(blk * RB, RB), RB), :])
        tiles = range(3 * NT_) if part is None else range(part * NT_, (part + 1) * NT_)
        for j in tiles:
            x = _w(xp[...])
            y = _dot(x, _w(wqkvb32[j * 64:(j + 1) * 64, :]), NT)
            if first:
                cur[j, HALO:HALO + RB, :] = y
                if j >= NT_:
                    cur[j, 0:HALO, :] = jnp.zeros((HALO, 128), F32)
            else:
                fresh[j] = y

    def b_rotate():
        for j in range(NT_, 3 * NT_):
            cur[j, 0:HALO, :] = cur[j, RB:RB + HALO, :]
        for j in range(3 * NT_):
            cur[j, HALO:HALO + RB, :] = fresh[j]
        ocur[...] = onew[...]

    def b_attend_rows(base, n, row0):
        src = cur
        q = [src[j, HALO + base:HALO + base + n, :] for j in range(NT_)]
        row = jax.lax.broadcasted_iota(jnp.int32, (n, 128), 0) + (row0 + base)
        half = WIN // 2
        step = DIL * half
        logits = [None] * WIN
        for w in range(half):
            o = HALO + base - DIL * w - step
            lo = hi = None
            for j in range(NT_):
                k = src[NT_ + j, o:o + n + step, :]
                a, b = q[j] * k[step:], q[j] * k[:n]
                lo = a if lo is None else lo + a
                hi = b if hi is None else hi + b
            for ww, s in ((w, lo), (w + half, hi)):
                s = s + pltpu.roll(s, 64, 1)
                s = s + pltpu.roll(s, 32, 1)
                s = s * (DB ** -0.5 * LOG2E)
                if ww:
                    s = jnp.where(row >= DIL * ww, s, MASK_VALUE * LOG2E)
                logits[ww] = s
        m = logits[0]
        for w in range(1, WIN):
            m = jnp.maximum(m, logits[w])
        e = [jnp.exp2(l - m) for l in logits]
        den = e[0]
        for w in range(1, WIN):
            den = den + e[w]
        r = _recip(den)
        outs = []
        for j in range(NT_):
            acc = None
            for w in range(half):
                o = HALO + base - DIL * w - step
                v = src[2 * NT_ + j, o:o + n + step, :]
                t = e[w] * v[step:] + e[w + half] * v[:n]
                acc = t if acc is None else acc + t
            outs.append(acc * r)
        return jnp.concatenate(outs, axis=1)

    def b_attend(blk, between=()):
        sub = cfg.get('sub', 64)
        between = list(between)
        for base in range(0, RB, sub):
            if between:
                between.pop(0)()
            onew[base:base + sub, :] = b_attend_rows(base, sub, blk * RB)
        for f in between:
            f()

    def b_output(blk, src):
        b_v[pl.ds(pl.multiple_of(blk * RB, RB), RB), :] = _dot(src[...], _w(wob32[...]))

    def qkv_weight(p, i):
        if cfg.get('nodma'):
            return
        rows = pl.ds(pl.multiple_of(p * PW, 128), PW)
        col = pl.multiple_of(p * 3 * PW, 128)
        w32[:, pl.ds(col + i * PW, PW)] = _pack(stage[i, rows, :].astype(F32).T.astype(BF16))

    def qkv_weights(p):
        for i in range(3):
            qkv_weight(p, i)

    def wait_qkv(p):
        if cfg.get('nodma'):
            return
        for c in qkv_copies(p):
            c.wait()

    c_xa0.wait()
    c_wqkvb[0].wait()
    n_early = cfg.get('x2_pos', 4)
    for p in range(n_early):
        for c in qkv_copies(p):
            c.start(priority=1)
    prep_wqkvb(0)
    c_wqkvb[1].wait()
    c_xa2.start(priority=1)
    prep_wqkvb(1)
    b_project(0, first=True, part=0)
    c_wqkvb[2].wait()
    for p in range(n_early, NP):
        for c in qkv_copies(p):
            c.start(priority=1)
    prep_wqkvb(2)
    b_project(0, first=True, part=1)
    c_wob.wait()
    b_project(0, first=True, part=2)
    if not cfg.get('nodma') and not cfg.get('nowo'):
        for c in c_wo:
            c.start(priority=1)
    if cfg.get('wob_pos', 2) == 0:
        prep_wob()
    b_project(1)
    if cfg.get('wob_pos', 2) == 1:
        prep_wob()
    b_attend(0)
    if cfg.get('wob_pos', 2) == 2:
        prep_wob()
    b_rotate()
    c_xa1.wait()

    def p1_step(k):
        for c in cfg.get('order', 'poatr'):
            if c == 'p':
                b_project(k + 1)
            elif c == 'o':
                b_output(k - 1, ocur)
            elif c == 'a':
                b_attend(k)
            elif c == 't':
                qkv_weights(k - 1)
            elif c == 'r':
                b_rotate()

    unroll = cfg.get('unroll', 1)

    def p1_body(i, carry):
        k0 = 1 + unroll * i

        @pl.when(k0 == XA1 // RB - 1)
        def _():
            c_xa2.wait()

        for u in range(unroll):
            wait_qkv(k0 + u - 1)
        for u in range(unroll):
            p1_step(k0 + u)
        return carry

    jax.lax.fori_loop(0, (NB - 2) // unroll, p1_body, 0)
    wait_qkv(NB - 2)
    wait_qkv(NB - 1)
    b_output(NB - 2, ocur)
    if cfg.get('batt_t', 0) < 0:
        b_attend(NB - 1)
    qkv_weights(NB - 2)
    qkv_weights(NB - 1)

    if cfg.get('stop_after_p1'):
        if not cfg.get('nowo'):
            for c in c_wo:
                c.wait()
        return
    mem_last = cfg.get('mem_last', True)
    out_mem_first = cfg.get('out_mem_first', True)
    X0, M0 = (0, SEG) if mem_last else (M, 0)
    h_ref[M0:M0 + M, :] = mem_ref[...].astype(F32)
    gate = gate_ref[...].astype(F32).reshape(1, D)
    lag_b, lag_e, lag_f = cfg.get('lags', (1, 4, 8))

    def segment(s, carry, first=False, static=False):
        off = s * SEG if first or static else pl.multiple_of(s * SEG, SEG)
        x = xa_v[pl.ds(off, SEG), :].astype(F32)
        h_ref[X0:X0 + SEG, :] = x
        r = jax.lax.broadcasted_iota(jnp.int32, (L, 2 * L), 0)
        c = jax.lax.broadcasted_iota(jnp.int32, (L, 2 * L), 1)
        isb = c >= L
        key = jnp.where(isb, c - L, c)
        if mem_last:
            allowed = (r >= SEG) | (key >= SEG) | (r >= key)
        else:
            allowed = (r < M) | (r >= key)
        st = [dict() for _ in range(NP)]
        acc = [None]

        def project(p):
            h = h_ref[...]
            b = p * 3 * PW
            nk = cfg.get('kouter', 1) if p == 0 and not first else 0
            if nk:
                y = None
                for kt in range(NT_):
                    t = _dot(h[:, kt * 128:(kt + 1) * 128],
                             _w(w32[kt * 64:(kt + 1) * 64, b:b + nk * PW]))
                    y = t if y is None else y + t
                parts = [y[:, i * PW:(i + 1) * PW] for i in range(nk)]
            else:
                parts = []
            parts += [_dot(h, _w(w32[:, b + i * PW:b + (i + 1) * PW])) for i in range(nk, 3)]
            st[p]['q'] = parts[0]
            st[p]['kb'] = _blockdiag(parts[1])
            st[p]['vb'] = _blockdiag(parts[2])

        def softmax(p):
            sc = _dot(st[p].pop('q'), st[p].pop('kb'), NT)
            t = jnp.where(allowed, sc * (DH ** -0.5 * LOG2E), MASK_VALUE * LOG2E)
            ma = jnp.max(jnp.where(isb, -jnp.inf, t), axis=1, keepdims=True)
            mb = jnp.max(jnp.where(isb, t, -jnp.inf), axis=1, keepdims=True)
            e = jnp.exp2(t - jnp.where(isb, mb, ma))
            sa = jnp.sum(jnp.where(isb, 0.0, e), axis=1, keepdims=True)
            sb = jnp.sum(jnp.where(isb, e, 0.0), axis=1, keepdims=True)
            st[p]['p'] = e * _recip(jnp.where(isb, sb, sa))

        def values(p):
            st[p]['o'] = _dot(st[p].pop('p'), st[p].pop('vb'))

        def output(p):
            if first:
                w = wo_stage[p * PW:(p + 1) * PW, :]
                wo32[p * (PW // 2):(p + 1) * (PW // 2), :] = _pack(w)
            else:
                w = _w(wo32[p * (PW // 2):(p + 1) * (PW // 2), :])
            o = st[p].pop('o')
            if mem_last and out_mem_first:
                o = jnp.concatenate([o[SEG:L], o[0:SEG]], axis=0)
            y = _dot(o, w)
            acc[0] = y if acc[0] is None else acc[0] + y

        nsteps = NP + (lag_e + 1 if first else lag_f)
        wo_t = cfg.get('wo_t', (nsteps - 1,))
        for t in range(nsteps):
            if t < NP:
                project(t)
            if first and t == cfg.get('batt_t', 0):
                b_attend(NB - 1)
            if first and t == cfg.get('bout_t', 16):
                b_output(NB - 1, onew)
            if 0 <= t - lag_b < NP:
                softmax(t - lag_b)
            if 0 <= t - lag_e < NP:
                values(t - lag_e)
            if not first and 0 <= t - lag_f < NP:
                output(t - lag_f)
            if first:
                for i, tw in enumerate(wo_t):
                    if t == tw and not cfg.get('nodma'):
                        c_wo[i].wait()
                    if t >= tw:
                        lo, hi = i * NP // nwo, (i + 1) * NP // nwo
                        per = -(-(hi - lo) // (nsteps - tw)) if tw < nsteps else hi - lo
                        for p in range(lo + (t - tw) * per, min(hi, lo + (t - tw + 1) * per)):
                            output(p)
        a = acc[0]
        if mem_last and not out_mem_first:
            a_mem, a_x = a[SEG:L], a[0:SEG]
        else:
            a_mem, a_x = a[0:M], a[M:L]
        h_ref[M0:M0 + M, :] = a_mem
        z = jnp.sum(x * gate, axis=1, keepdims=True)
        g = 1.0 / (1.0 + jnp.exp(-z))
        y = g * a_x + (1.0 - g) * b_v[pl.ds(off, SEG), :]
        out_v[pl.ds(off, SEG), :] = y.astype(out_v.dtype)
        pltpu.make_async_copy(out_v.at[pl.ds(off, SEG), :], out_hbm.at[pl.ds(off, SEG), :],
                              sem_out.at[0]).start()
        return carry

    nseg = cfg.get('nseg', NSEG)
    if cfg.get('peel', True):
        segment(0, 0, first=True)
        start = 1
    else:
        b_attend(NB - 1)
        b_output(NB - 1, onew)
        for c in c_wo:
            c.wait()
        for p in range(NP):
            wo32[p * (PW // 2):(p + 1) * (PW // 2), :] = _pack(wo_stage[p * PW:(p + 1) * PW, :])
        start = 0
    su = cfg.get('seg_unroll', 3)
    if su > 1:
        while (nseg - start) % su:
            segment(start, 0, static=True)
            start += 1

        def segments(i, carry):
            for u in range(su):
                segment(start + i * su + u, carry)
            return carry
        jax.lax.fori_loop(0, (nseg - start) // su, segments, 0)
    elif nseg > start:
        jax.lax.fori_loop(start, nseg, segment, 0)
    n_out = max(nseg, start)
    if n_out:
        pltpu.make_async_copy(out_v.at[0:n_out * SEG, :], out_hbm.at[0:n_out * SEG, :],
                              sem_out.at[0]).wait()


def _forward(cfg, A_x, A_mem0, A_Wq, A_Wk, A_Wv, A_Wo, B_wqkv, B_wo, gate_w):
    def wt(w):
        return jnp.transpose(w, (1, 2, 0)).reshape(H * DH, D)

    hbm = pl.BlockSpec(memory_space=pl.ANY)
    vmem = pl.BlockSpec(memory_space=pltpu.VMEM)
    out = pl.pallas_call(
        functools.partial(_kernel, cfg),
        out_shape=jax.ShapeDtypeStruct((S, D), BF16),
        in_specs=[hbm, vmem, hbm, hbm, hbm, hbm, hbm, hbm, vmem],
        out_specs=hbm,
        scratch_shapes=[
            pltpu.VMEM((S, D), BF16),
            pltpu.VMEM((S, D), BF16),
            pltpu.VMEM((S, D), F32),
            pltpu.VMEM((L, D), F32),
            pltpu.VMEM((3, H * DH, D), BF16),
            pltpu.VMEM((H * DH, D), BF16),
            pltpu.VMEM((D // 2, 3 * H * DH), U32),
            pltpu.VMEM((H * DH // 2, D), U32),
            pltpu.VMEM((D, 3 * D), BF16),
            pltpu.VMEM((D, D), BF16),
            pltpu.VMEM((3 * D // 2, D), U32),
            pltpu.VMEM((D // 2, D), U32),
            pltpu.VMEM((NT_, 3 * D, 128), F32),
            pltpu.VMEM((3 * NT_, RB, 128), F32),
            pltpu.VMEM((3 * NT_, HALO + RB, 128), F32),
            pltpu.VMEM((RB, D), F32),
            pltpu.VMEM((RB, D), F32),
            pltpu.VMEM((2, RB // 2, D), U32),
            pltpu.SemaphoreType.DMA((NP,)),
            pltpu.SemaphoreType.DMA((4,)),
            pltpu.SemaphoreType.DMA((4 + cfg.get('nwo', 1),)),
            pltpu.SemaphoreType.DMA((1,)),
        ],
        compiler_params=pltpu.CompilerParams(vmem_limit_bytes=120 * 1024 * 1024,
                                             disable_bounds_checks=True),
    )(A_x.reshape(S, D), A_mem0.reshape(M, D), wt(A_Wq), wt(A_Wk), wt(A_Wv),
      A_Wo.reshape(H * DH, D), B_wqkv, B_wo, gate_w)
    return out.reshape(1, S, D)


@functools.partial(jax.jit, static_argnames=("A_seg_len",))
def pallas_gated_mix__memory_aug_recurrent_mem_tr__sliding_local_dilated__prompt_kernel(
    A_x: jax.Array,
    A_mem0: jax.Array,
    A_Wq: jax.Array,
    A_Wk: jax.Array,
    A_Wv: jax.Array,
    A_Wo: jax.Array,
    A_seg_len: int,
    B_x: jax.Array,
    B_wqkv: jax.Array,
    B_wo: jax.Array,
    gate_w: jax.Array,
):
    del B_x
    assert A_seg_len == SEG
    assert A_x.shape == (1, S, D) and A_Wq.shape == (D, H, DH) and A_mem0.shape == (1, M, D)
    return _forward({}, A_x, A_mem0, A_Wq, A_Wk, A_Wv, A_Wo, B_wqkv, B_wo, gate_w)
```

```python
import functools

import jax
import jax.numpy as jnp
from jax.experimental import pallas as pl
from jax.experimental.pallas import tpu as pltpu

F32 = jnp.float32
BF16 = jnp.bfloat16
U32 = jnp.uint32

S = 2048
D = 640
NT_ = D // 128
MASK_VALUE = -1e9
LOG2E = 1.4426950408889634
H = 32
DH = 192
M = 8
SEG = 32
L = M + SEG
NSEG = S // SEG
NP = H // 2
PW = 2 * DH
LAG_S, LAG_V, LAG_O = 1, 4, 8
SEG_UNROLL = 3
HB = 32
DB = D // HB
WIN = 8
DIL = 2
RB = 128
NB = S // RB
SUB = 64
HALO = 16
XA0 = 256
XA1 = 768
EARLY_PAIRS = 4

NN = (((1,), (0,)), ((), ()))
NT = (((1,), (1,)), ((), ()))


def _dot(a, b, dims=NN):
    return jax.lax.dot_general(a, b, dims, preferred_element_type=F32)


def _w(x):
    return pltpu.bitcast(x, BF16)


def _pack(x):
    return pltpu.bitcast(x, U32)


def _recip(den):
    r = pl.reciprocal(den, approx=True)
    return r * (2.0 - den * r)


def _blockdiag(t):
    lo = jax.lax.broadcasted_iota(jnp.int32, (L, 128), 1) < 64
    z = jnp.zeros((L, 128), F32)
    t0, t1, t2 = t[:, 0:128], t[:, 128:256], t[:, 256:384]
    top = jnp.concatenate([t0, jnp.where(lo, t1, 0.0), z], axis=1)
    bot = jnp.concatenate([z, jnp.where(lo, 0.0, t1), t2], axis=1)
    return jnp.concatenate([top, bot], axis=0).astype(BF16)


def _kernel(x_hbm, mem_hbm, wq_hbm, wk_hbm, wv_hbm, wo_hbm, wqkvb_hbm, wob_hbm, gate_hbm,
            out_hbm,
            x_v, out_v, b_v, h_ref, mem_v, gate_v,
            qkv_stage, wo_stage, w32, wo32,
            wqkvb_v, wob_v, wqkvb32, wob32, prep, fresh, cur, onew, ocur, x32,
            sem_qkv, sem_in, sem_out):
    def qkv_copies(p):
        rows = pl.ds(pl.multiple_of(p * PW, 128), PW)
        return [pltpu.make_async_copy(src.at[rows, :], qkv_stage.at[i, rows, :], sem_qkv.at[p])
                for i, src in enumerate((wq_hbm, wk_hbm, wv_hbm))]

    def start_qkv(pairs):
        for p in pairs:
            for c in qkv_copies(p):
                c.start(priority=1)

    def wait_qkv(p):
        for c in qkv_copies(p):
            c.wait()

    c_wqkvb = [pltpu.make_async_copy(wqkvb_hbm.at[:, i * D:(i + 1) * D],
                                     wqkvb_v.at[:, i * D:(i + 1) * D], sem_in.at[i])
               for i in range(3)]
    c_x = [pltpu.make_async_copy(x_hbm.at[lo:hi, :], x_v.at[lo:hi, :], sem_in.at[3 + i])
           for i, (lo, hi) in enumerate(((0, XA0), (XA0, XA1), (XA1, S)))]
    c_wob = pltpu.make_async_copy(wob_hbm, wob_v, sem_in.at[6])
    c_wo = pltpu.make_async_copy(wo_hbm, wo_stage, sem_in.at[7])
    c_mem = pltpu.make_async_copy(mem_hbm, mem_v, sem_in.at[8])
    c_gate = pltpu.make_async_copy(gate_hbm, gate_v, sem_in.at[9])
    c_x[0].start()
    for c in c_wqkvb:
        c.start()
    for c in (c_wob, c_x[1], c_mem, c_gate):
        c.start(priority=1)

    def prep_wqkvb(part):
        for c in range(part * NT_, (part + 1) * NT_):
            t = wqkvb_v[:, c * 128:(c + 1) * 128].astype(F32).T
            for kt in range(NT_):
                prep[kt, c * 128:(c + 1) * 128, :] = t[:, kt * 128:(kt + 1) * 128]
        for d in range(DB):
            rows = jnp.concatenate(
                [prep[kt, pl.ds(part * D + d, HB, stride=DB), :] for kt in range(NT_)], axis=1)
            r0 = (part * D + d * HB) // 2
            wqkvb32[r0:r0 + HB // 2, :] = _pack(rows.astype(BF16))

    def prep_wob():
        for kt in range(NT_):
            prep[kt, 0:D, :] = wob_v[:, kt * 128:(kt + 1) * 128].astype(F32)
        for d in range(DB):
            rows = jnp.concatenate(
                [prep[kt, pl.ds(d, HB, stride=DB), :] for kt in range(NT_)], axis=1)
            wob32[d * (HB // 2):(d + 1) * (HB // 2), :] = _pack(rows.astype(BF16))

    def b_project(blk, part=None):
        xp = x32.at[0 if part is None else 1]
        if not part:
            xp[...] = _pack(x_v[pl.ds(pl.multiple_of(blk * RB, RB), RB), :])
        tiles = range(3 * NT_) if part is None else range(part * NT_, (part + 1) * NT_)
        for j in tiles:
            y = _dot(_w(xp[...]), _w(wqkvb32[j * 64:(j + 1) * 64, :]), NT)
            if part is None:
                fresh[j] = y
            else:
                cur[j, HALO:HALO + RB, :] = y
                if j >= NT_:
                    cur[j, 0:HALO, :] = jnp.zeros((HALO, 128), F32)

    def b_rotate():
        for j in range(NT_, 3 * NT_):
            cur[j, 0:HALO, :] = cur[j, RB:RB + HALO, :]
        for j in range(3 * NT_):
            cur[j, HALO:HALO + RB, :] = fresh[j]
        ocur[...] = onew[...]

    def b_attend_rows(base, n, row0):
        q = [cur[j, HALO + base:HALO + base + n, :] for j in range(NT_)]
        row = jax.lax.broadcasted_iota(jnp.int32, (n, 128), 0) + (row0 + base)
        half = WIN // 2
        step = DIL * half
        logits = [None] * WIN
        for w in range(half):
            o = HALO + base - DIL * w - step
            lo = hi = None
            for j in range(NT_):
                k = cur[NT_ + j, o:o + n + step, :]
                a, b = q[j] * k[step:], q[j] * k[:n]
                lo = a if lo is None else lo + a
                hi = b if hi is None else hi + b
            for ww, s in ((w, lo), (w + half, hi)):
                s = s + pltpu.roll(s, 64, 1)
                s = s + pltpu.roll(s, 32, 1)
                s = s * (DB ** -0.5 * LOG2E)
                if ww:
                    s = jnp.where(row >= DIL * ww, s, MASK_VALUE * LOG2E)
                logits[ww] = s
        m = logits[0]
        for w in range(1, WIN):
            m = jnp.maximum(m, logits[w])
        e = [jnp.exp2(l - m) for l in logits]
        den = e[0]
        for w in range(1, WIN):
            den = den + e[w]
        r = _recip(den)
        outs = []
        for j in range(NT_):
            acc = None
            for w in range(half):
                o = HALO + base - DIL * w - step
                v = cur[2 * NT_ + j, o:o + n + step, :]
                t = e[w] * v[step:] + e[w + half] * v[:n]
                acc = t if acc is None else acc + t
            outs.append(acc * r)
        return jnp.concatenate(outs, axis=1)

    def b_attend(blk):
        for base in range(0, RB, SUB):
            onew[base:base + SUB, :] = b_attend_rows(base, SUB, blk * RB)

    def b_output(blk, src):
        b_v[pl.ds(pl.multiple_of(blk * RB, RB), RB), :] = _dot(src[...], _w(wob32[...]))

    def a_qkv_weights(p):
        rows = pl.ds(pl.multiple_of(p * PW, 128), PW)
        col = pl.multiple_of(p * 3 * PW, 128)
        for i in range(3):
            w32[:, pl.ds(col + i * PW, PW)] = _pack(
                qkv_stage[i, rows, :].astype(F32).T.astype(BF16))

    c_x[0].wait()
    c_wqkvb[0].wait()
    start_qkv(range(EARLY_PAIRS))
    prep_wqkvb(0)
    c_wqkvb[1].wait()
    c_x[2].start(priority=1)
    prep_wqkvb(1)
    b_project(0, part=0)
    c_wqkvb[2].wait()
    start_qkv(range(EARLY_PAIRS, NP))
    prep_wqkvb(2)
    b_project(0, part=1)
    c_wob.wait()
    b_project(0, part=2)
    c_wo.start(priority=1)
    b_project(1)
    b_attend(0)
    prep_wob()
    b_rotate()
    c_x[1].wait()
    c_mem.wait()
    c_gate.wait()

    def b_step(k, carry):
        @pl.when(k == XA1 // RB - 1)
        def _():
            c_x[2].wait()

        wait_qkv(k - 1)
        b_project(k + 1)
        b_output(k - 1, ocur)
        b_attend(k)
        a_qkv_weights(k - 1)
        b_rotate()
        return carry

    jax.lax.fori_loop(1, NB - 1, b_step, 0)
    wait_qkv(NB - 2)
    wait_qkv(NB - 1)
    b_output(NB - 2, ocur)
    a_qkv_weights(NB - 2)
    a_qkv_weights(NB - 1)

    h_ref[SEG:L, :] = mem_v[...].astype(F32)
    gate = gate_v[...].astype(F32).reshape(1, D)

    def segment(s, first=False):
        off = s * SEG if first else pl.multiple_of(s * SEG, SEG)
        x = x_v[pl.ds(off, SEG), :].astype(F32)
        h_ref[0:SEG, :] = x
        r = jax.lax.broadcasted_iota(jnp.int32, (L, 2 * L), 0)
        c = jax.lax.broadcasted_iota(jnp.int32, (L, 2 * L), 1)
        isb = c >= L
        key = jnp.where(isb, c - L, c)
        allowed = (r >= SEG) | (key >= SEG) | (r >= key)
        st = [dict() for _ in range(NP)]
        acc = [None]

        def project(p):
            h = h_ref[...]
            b = p * 3 * PW
            if p == 0 and not first:
                q = None
                for kt in range(NT_):
                    t = _dot(h[:, kt * 128:(kt + 1) * 128],
                             _w(w32[kt * 64:(kt + 1) * 64, b:b + PW]))
                    q = t if q is None else q + t
            else:
                q = _dot(h, _w(w32[:, b:b + PW]))
            st[p]['q'] = q
            st[p]['kb'] = _blockdiag(_dot(h, _w(w32[:, b + PW:b + 2 * PW])))
            st[p]['vb'] = _blockdiag(_dot(h, _w(w32[:, b + 2 * PW:b + 3 * PW])))

        def softmax(p):
            sc = _dot(st[p].pop('q'), st[p].pop('kb'), NT)
            t = jnp.where(allowed, sc * (DH ** -0.5 * LOG2E), MASK_VALUE * LOG2E)
            ma = jnp.max(jnp.where(isb, -jnp.inf, t), axis=1, keepdims=True)
            mb = jnp.max(jnp.where(isb, t, -jnp.inf), axis=1, keepdims=True)
            e = jnp.exp2(t - jnp.where(isb, mb, ma))
            sa = jnp.sum(jnp.where(isb, 0.0, e), axis=1, keepdims=True)
            sb = jnp.sum(jnp.where(isb, e, 0.0), axis=1, keepdims=True)
            st[p]['p'] = e * _recip(jnp.where(isb, sb, sa))

        def values(p):
            st[p]['o'] = _dot(st[p].pop('p'), st[p].pop('vb'))

        def output(p):
            if first:
                w = wo_stage[p * PW:(p + 1) * PW, :]
                wo32[p * (PW // 2):(p + 1) * (PW // 2), :] = _pack(w)
            else:
                w = _w(wo32[p * (PW // 2):(p + 1) * (PW // 2), :])
            o = st[p].pop('o')
            y = _dot(jnp.concatenate([o[SEG:L], o[0:SEG]], axis=0), w)
            acc[0] = y if acc[0] is None else acc[0] + y

        for t in range(NP + (LAG_V if first else LAG_O)):
            if t < NP:
                project(t)
            if first and t == 0:
                b_attend(NB - 1)
            if first and t == NP:
                b_output(NB - 1, onew)
            if 0 <= t - LAG_S < NP:
                softmax(t - LAG_S)
            if 0 <= t - LAG_V < NP:
                values(t - LAG_V)
            if not first and 0 <= t - LAG_O < NP:
                output(t - LAG_O)
        if first:
            c_wo.wait()
            for p in range(NP):
                output(p)
        a = acc[0]
        h_ref[SEG:L, :] = a[0:M]
        z = jnp.sum(x * gate, axis=1, keepdims=True)
        g = 1.0 / (1.0 + jnp.exp(-z))
        y = g * a[M:L] + (1.0 - g) * b_v[pl.ds(off, SEG), :]
        out_v[pl.ds(off, SEG), :] = y.astype(out_v.dtype)
        pltpu.make_async_copy(out_v.at[pl.ds(off, SEG), :], out_hbm.at[pl.ds(off, SEG), :],
                              sem_out.at[0]).start()

    segment(0, first=True)

    def segments(i, carry):
        for u in range(SEG_UNROLL):
            segment(1 + i * SEG_UNROLL + u)
        return carry

    jax.lax.fori_loop(0, (NSEG - 1) // SEG_UNROLL, segments, 0)
    pltpu.make_async_copy(out_v, out_hbm, sem_out.at[0]).wait()


@functools.partial(jax.jit, static_argnames=("A_seg_len",))
def pallas_gated_mix__memory_aug_recurrent_mem_tr__sliding_local_dilated__prompt_kernel(
    A_x: jax.Array,
    A_mem0: jax.Array,
    A_Wq: jax.Array,
    A_Wk: jax.Array,
    A_Wv: jax.Array,
    A_Wo: jax.Array,
    A_seg_len: int,
    B_x: jax.Array,
    B_wqkv: jax.Array,
    B_wo: jax.Array,
    gate_w: jax.Array,
):
    del B_x
    assert A_seg_len == SEG and (NSEG - 1) % SEG_UNROLL == 0
    assert A_x.shape == (1, S, D) and A_Wq.shape == (D, H, DH) and A_mem0.shape == (1, M, D)

    def wt(w):
        return jnp.transpose(w, (1, 2, 0)).reshape(H * DH, D)

    hbm = pl.BlockSpec(memory_space=pl.ANY)
    out = pl.pallas_call(
        _kernel,
        out_shape=jax.ShapeDtypeStruct((S, D), BF16),
        in_specs=[hbm] * 9,
        out_specs=hbm,
        scratch_shapes=[
            pltpu.VMEM((S, D), BF16),
            pltpu.VMEM((S, D), BF16),
            pltpu.VMEM((S, D), F32),
            pltpu.VMEM((L, D), F32),
            pltpu.VMEM((M, D), BF16),
            pltpu.VMEM((D,), BF16),
            pltpu.VMEM((3, H * DH, D), BF16),
            pltpu.VMEM((H * DH, D), BF16),
            pltpu.VMEM((D // 2, 3 * H * DH), U32),
            pltpu.VMEM((H * DH // 2, D), U32),
            pltpu.VMEM((D, 3 * D), BF16),
            pltpu.VMEM((D, D), BF16),
            pltpu.VMEM((3 * D // 2, D), U32),
            pltpu.VMEM((D // 2, D), U32),
            pltpu.VMEM((NT_, 3 * D, 128), F32),
            pltpu.VMEM((3 * NT_, RB, 128), F32),
            pltpu.VMEM((3 * NT_, HALO + RB, 128), F32),
            pltpu.VMEM((RB, D), F32),
            pltpu.VMEM((RB, D), F32),
            pltpu.VMEM((2, RB // 2, D), U32),
            pltpu.SemaphoreType.DMA((NP,)),
            pltpu.SemaphoreType.DMA((10,)),
            pltpu.SemaphoreType.DMA((1,)),
        ],
        compiler_params=pltpu.CompilerParams(vmem_limit_bytes=120 * 1024 * 1024,
                                             disable_bounds_checks=True),
    )(A_x.reshape(S, D), A_mem0.reshape(M, D), wt(A_Wq), wt(A_Wk), wt(A_Wv),
      A_Wo.reshape(H * DH, D), B_wqkv, B_wo, gate_w)
    return out.reshape(1, S, D)
```

```python
import functools

import jax
import jax.numpy as jnp
from jax.experimental import pallas as pl
from jax.experimental.pallas import tpu as pltpu

F32 = jnp.float32
BF16 = jnp.bfloat16
U32 = jnp.uint32

S = 2048
D = 640
NT_ = D // 128
MASK_VALUE = -1e9
LOG2E = 1.4426950408889634
H = 32
DH = 192
M = 8
SEG = 32
L = M + SEG
NSEG = S // SEG
NP = H // 2
PW = 2 * DH
LAG_S, LAG_V, LAG_O = 1, 4, 8
SEG_UNROLL = 3
HB = 32
DB = D // HB
WIN = 8
DIL = 2
RB = 128
NB = S // RB
SUB = 64
HALO = 16
XA0 = 256
XA1 = 768
EARLY_PAIRS = 4
WO_SPLIT = 10

NN = (((1,), (0,)), ((), ()))
NT = (((1,), (1,)), ((), ()))


def _dot(a, b, dims=NN):
    return jax.lax.dot_general(a, b, dims, preferred_element_type=F32)


def _w(x):
    return pltpu.bitcast(x, BF16)


def _pack(x):
    return pltpu.bitcast(x, U32)


def _recip(den):
    r = pl.reciprocal(den, approx=True)
    return r * (2.0 - den * r)


def _blockdiag(t):
    lo = jax.lax.broadcasted_iota(jnp.int32, (L, 128), 1) < 64
    z = jnp.zeros((L, 128), F32)
    t0, t1, t2 = t[:, 0:128], t[:, 128:256], t[:, 256:384]
    top = jnp.concatenate([t0, jnp.where(lo, t1, 0.0), z], axis=1)
    bot = jnp.concatenate([z, jnp.where(lo, 0.0, t1), t2], axis=1)
    return jnp.concatenate([top, bot], axis=0).astype(BF16)


def _kernel(x_hbm, mem_hbm, wq_hbm, wk_hbm, wv_hbm, wo_hbm, wqkvb_hbm, wob_hbm, gate_hbm,
            out_hbm,
            x_v, out_v, b_v, h_ref, mem_v, gate_v,
            qkv_stage, wo_stage, w32, wo32,
            wqkvb_v, wob_v, wqkvb32, wob32, prep, fresh, cur, onew, ocur, x32,
            sem_qkv, sem_in, sem_out):
    def qkv_copies(p):
        rows = pl.ds(pl.multiple_of(p * PW, 128), PW)
        return [pltpu.make_async_copy(src.at[rows, :], qkv_stage.at[i, rows, :], sem_qkv.at[p])
                for i, src in enumerate((wq_hbm, wk_hbm, wv_hbm))]

    def start_qkv(pairs):
        for p in pairs:
            for c in qkv_copies(p):
                c.start(priority=1)

    def wait_qkv(p):
        for c in qkv_copies(p):
            c.wait()

    c_wqkvb = [pltpu.make_async_copy(wqkvb_hbm.at[:, i * D:(i + 1) * D],
                                     wqkvb_v.at[:, i * D:(i + 1) * D], sem_in.at[i])
               for i in range(3)]
    c_x = [pltpu.make_async_copy(x_hbm.at[lo:hi, :], x_v.at[lo:hi, :], sem_in.at[3 + i])
           for i, (lo, hi) in enumerate(((0, XA0), (XA0, XA1), (XA1, S)))]
    c_wob = pltpu.make_async_copy(wob_hbm, wob_v, sem_in.at[6])
    c_wo = [pltpu.make_async_copy(wo_hbm.at[lo * PW:hi * PW, :], wo_stage.at[lo * PW:hi * PW, :],
                                  sem_in.at[sem])
            for lo, hi, sem in ((0, WO_SPLIT, 7), (WO_SPLIT, NP, 10))]
    c_mem = pltpu.make_async_copy(mem_hbm, mem_v, sem_in.at[8])
    c_gate = pltpu.make_async_copy(gate_hbm, gate_v, sem_in.at[9])
    c_x[0].start()
    for c in c_wqkvb:
        c.start()
    for c in (c_wob, c_x[1], c_mem, c_gate):
        c.start(priority=1)

    def prep_wqkvb(part):
        for c in range(part * NT_, (part + 1) * NT_):
            t = wqkvb_v[:, c * 128:(c + 1) * 128].astype(F32).T
            for kt in range(NT_):
                prep[kt, c * 128:(c + 1) * 128, :] = t[:, kt * 128:(kt + 1) * 128]
        for d in range(DB):
            rows = jnp.concatenate(
                [prep[kt, pl.ds(part * D + d, HB, stride=DB), :] for kt in range(NT_)], axis=1)
            r0 = (part * D + d * HB) // 2
            wqkvb32[r0:r0 + HB // 2, :] = _pack(rows.astype(BF16))

    def prep_wob():
        for kt in range(NT_):
            prep[kt, 0:D, :] = wob_v[:, kt * 128:(kt + 1) * 128].astype(F32)
        for d in range(DB):
            rows = jnp.concatenate(
                [prep[kt, pl.ds(d, HB, stride=DB), :] for kt in range(NT_)], axis=1)
            wob32[d * (HB // 2):(d + 1) * (HB // 2), :] = _pack(rows.astype(BF16))

    def b_project(blk, part=None):
        xp = x32.at[0 if part is None else 1]
        if not part:
            xp[...] = _pack(x_v[pl.ds(pl.multiple_of(blk * RB, RB), RB), :])
        tiles = range(3 * NT_) if part is None else range(part * NT_, (part + 1) * NT_)
        for j in tiles:
            y = _dot(_w(xp[...]), _w(wqkvb32[j * 64:(j + 1) * 64, :]), NT)
            if part is None:
                fresh[j] = y
            else:
                cur[j, HALO:HALO + RB, :] = y
                if j >= NT_:
                    cur[j, 0:HALO, :] = jnp.zeros((HALO, 128), F32)

    def b_rotate():
        for j in range(NT_, 3 * NT_):
            cur[j, 0:HALO, :] = cur[j, RB:RB + HALO, :]
        for j in range(3 * NT_):
            cur[j, HALO:HALO + RB, :] = fresh[j]
        ocur[...] = onew[...]

    def b_attend_rows(base, n, row0):
        q = [cur[j, HALO + base:HALO + base + n, :] for j in range(NT_)]
        row = jax.lax.broadcasted_iota(jnp.int32, (n, 128), 0) + (row0 + base)
        half = WIN // 2
        step = DIL * half
        logits = [None] * WIN
        for w in range(half):
            o = HALO + base - DIL * w - step
            lo = hi = None
            for j in range(NT_):
                k = cur[NT_ + j, o:o + n + step, :]
                a, b = q[j] * k[step:], q[j] * k[:n]
                lo = a if lo is None else lo + a
                hi = b if hi is None else hi + b
            for ww, s in ((w, lo), (w + half, hi)):
                s = s + pltpu.roll(s, 64, 1)
                s = s + pltpu.roll(s, 32, 1)
                s = s * (DB ** -0.5 * LOG2E)
                if ww:
                    s = jnp.where(row >= DIL * ww, s, MASK_VALUE * LOG2E)
                logits[ww] = s
        m = logits[0]
        for w in range(1, WIN):
            m = jnp.maximum(m, logits[w])
        e = [jnp.exp2(l - m) for l in logits]
        den = e[0]
        for w in range(1, WIN):
            den = den + e[w]
        r = _recip(den)
        outs = []
        for j in range(NT_):
            acc = None
            for w in range(half):
                o = HALO + base - DIL * w - step
                v = cur[2 * NT_ + j, o:o + n + step, :]
                t = e[w] * v[step:] + e[w + half] * v[:n]
                acc = t if acc is None else acc + t
            outs.append(acc * r)
        return jnp.concatenate(outs, axis=1)

    def b_attend(blk):
        for base in range(0, RB, SUB):
            onew[base:base + SUB, :] = b_attend_rows(base, SUB, blk * RB)

    def b_output(blk, src):
        b_v[pl.ds(pl.multiple_of(blk * RB, RB), RB), :] = _dot(src[...], _w(wob32[...]))

    def a_qkv_weights(p):
        rows = pl.ds(pl.multiple_of(p * PW, 128), PW)
        col = pl.multiple_of(p * 3 * PW, 128)
        for i in range(3):
            w32[:, pl.ds(col + i * PW, PW)] = _pack(
                qkv_stage[i, rows, :].astype(F32).T.astype(BF16))

    c_x[0].wait()
    c_wqkvb[0].wait()
    start_qkv(range(EARLY_PAIRS))
    prep_wqkvb(0)
    c_wqkvb[1].wait()
    c_x[2].start(priority=1)
    prep_wqkvb(1)
    b_project(0, part=0)
    c_wqkvb[2].wait()
    start_qkv(range(EARLY_PAIRS, NP))
    prep_wqkvb(2)
    b_project(0, part=1)
    c_wob.wait()
    b_project(0, part=2)
    for c in c_wo:
        c.start(priority=1)
    b_project(1)
    b_attend(0)
    prep_wob()
    b_rotate()
    c_x[1].wait()
    c_mem.wait()
    c_gate.wait()

    def b_step(k, carry):
        @pl.when(k == XA1 // RB - 1)
        def _():
            c_x[2].wait()

        wait_qkv(k - 1)
        b_project(k + 1)
        b_output(k - 1, ocur)
        b_attend(k)
        a_qkv_weights(k - 1)
        b_rotate()
        return carry

    jax.lax.fori_loop(1, NB - 1, b_step, 0)

    h_ref[SEG:L, :] = mem_v[...].astype(F32)
    gate = gate_v[...].astype(F32).reshape(1, D)

    def segment(s, first=False):
        off = s * SEG if first else pl.multiple_of(s * SEG, SEG)
        x = x_v[pl.ds(off, SEG), :].astype(F32)
        h_ref[0:SEG, :] = x
        r = jax.lax.broadcasted_iota(jnp.int32, (L, 2 * L), 0)
        c = jax.lax.broadcasted_iota(jnp.int32, (L, 2 * L), 1)
        isb = c >= L
        key = jnp.where(isb, c - L, c)
        allowed = (r >= SEG) | (key >= SEG) | (r >= key)
        st = [dict() for _ in range(NP)]
        acc = [None]

        def project(p):
            h = h_ref[...]
            b = p * 3 * PW
            if p == 0 and not first:
                q = None
                for kt in range(NT_):
                    t = _dot(h[:, kt * 128:(kt + 1) * 128],
                             _w(w32[kt * 64:(kt + 1) * 64, b:b + PW]))
                    q = t if q is None else q + t
            else:
                q = _dot(h, _w(w32[:, b:b + PW]))
            st[p]['q'] = q
            st[p]['kb'] = _blockdiag(_dot(h, _w(w32[:, b + PW:b + 2 * PW])))
            st[p]['vb'] = _blockdiag(_dot(h, _w(w32[:, b + 2 * PW:b + 3 * PW])))

        def softmax(p):
            sc = _dot(st[p].pop('q'), st[p].pop('kb'), NT)
            t = jnp.where(allowed, sc * (DH ** -0.5 * LOG2E), MASK_VALUE * LOG2E)
            ma = jnp.max(jnp.where(isb, -jnp.inf, t), axis=1, keepdims=True)
            mb = jnp.max(jnp.where(isb, t, -jnp.inf), axis=1, keepdims=True)
            e = jnp.exp2(t - jnp.where(isb, mb, ma))
            sa = jnp.sum(jnp.where(isb, 0.0, e), axis=1, keepdims=True)
            sb = jnp.sum(jnp.where(isb, e, 0.0), axis=1, keepdims=True)
            st[p]['p'] = e * _recip(jnp.where(isb, sb, sa))

        def values(p):
            st[p]['o'] = _dot(st[p].pop('p'), st[p].pop('vb'))

        def output(p):
            if first:
                w = wo_stage[p * PW:(p + 1) * PW, :]
                wo32[p * (PW // 2):(p + 1) * (PW // 2), :] = _pack(w)
            else:
                w = _w(wo32[p * (PW // 2):(p + 1) * (PW // 2), :])
            o = st[p].pop('o')
            y = _dot(jnp.concatenate([o[SEG:L], o[0:SEG]], axis=0), w)
            acc[0] = y if acc[0] is None else acc[0] + y

        for t in range(NP + (LAG_V + 1 if first else LAG_O)):
            if t < NP:
                project(t)
            if first and t == 0:
                b_attend(NB - 1)
            if first and t == NP:
                b_output(NB - 1, onew)
            if 0 <= t - LAG_S < NP:
                softmax(t - LAG_S)
            if 0 <= t - LAG_V < NP:
                values(t - LAG_V)
            if not first and 0 <= t - LAG_O < NP:
                output(t - LAG_O)
            if first and t >= NP + 2:
                if t == NP + 2:
                    c_wo[0].wait()
                j = t - (NP + 2)
                for p in range(4 * j, min(4 * j + 4, WO_SPLIT)):
                    output(p)
        if first:
            c_wo[1].wait()
            for p in range(WO_SPLIT, NP):
                output(p)
        a = acc[0]
        h_ref[SEG:L, :] = a[0:M]
        z = jnp.sum(x * gate, axis=1, keepdims=True)
        g = 1.0 / (1.0 + jnp.exp(-z))
        y = g * a[M:L] + (1.0 - g) * b_v[pl.ds(off, SEG), :]
        out_v[pl.ds(off, SEG), :] = y.astype(out_v.dtype)
        pltpu.make_async_copy(out_v.at[pl.ds(off, SEG), :], out_hbm.at[pl.ds(off, SEG), :],
                              sem_out.at[0]).start()

    def first_segment(i, carry):
        wait_qkv(NB - 2)
        wait_qkv(NB - 1)
        b_output(NB - 2, ocur)
        a_qkv_weights(NB - 2)
        a_qkv_weights(NB - 1)
        segment(0, first=True)
        return carry

    jax.lax.fori_loop(0, pl.program_id(0) + 1, first_segment, 0)

    def segments(i, carry):
        for u in range(SEG_UNROLL):
            segment(1 + i * SEG_UNROLL + u)
        return carry

    jax.lax.fori_loop(0, (NSEG - 1) // SEG_UNROLL, segments, 0)
    pltpu.make_async_copy(out_v, out_hbm, sem_out.at[0]).wait()


@functools.partial(jax.jit, static_argnames=("A_seg_len",))
def pallas_gated_mix__memory_aug_recurrent_mem_tr__sliding_local_dilated__prompt_kernel(
    A_x: jax.Array,
    A_mem0: jax.Array,
    A_Wq: jax.Array,
    A_Wk: jax.Array,
    A_Wv: jax.Array,
    A_Wo: jax.Array,
    A_seg_len: int,
    B_x: jax.Array,
    B_wqkv: jax.Array,
    B_wo: jax.Array,
    gate_w: jax.Array,
):
    del B_x
    assert A_seg_len == SEG and (NSEG - 1) % SEG_UNROLL == 0
    assert A_x.shape == (1, S, D) and A_Wq.shape == (D, H, DH) and A_mem0.shape == (1, M, D)

    def wt(w):
        return jnp.transpose(w, (1, 2, 0)).reshape(H * DH, D)

    hbm = pl.BlockSpec(memory_space=pl.ANY)
    out = pl.pallas_call(
        _kernel,
        out_shape=jax.ShapeDtypeStruct((S, D), BF16),
        in_specs=[hbm] * 9,
        out_specs=hbm,
        grid=(1,),
        scratch_shapes=[
            pltpu.VMEM((S, D), BF16),
            pltpu.VMEM((S, D), BF16),
            pltpu.VMEM((S, D), F32),
            pltpu.VMEM((L, D), F32),
            pltpu.VMEM((M, D), BF16),
            pltpu.VMEM((D,), BF16),
            pltpu.VMEM((3, H * DH, D), BF16),
            pltpu.VMEM((H * DH, D), BF16),
            pltpu.VMEM((D // 2, 3 * H * DH), U32),
            pltpu.VMEM((H * DH // 2, D), U32),
            pltpu.VMEM((D, 3 * D), BF16),
            pltpu.VMEM((D, D), BF16),
            pltpu.VMEM((3 * D // 2, D), U32),
            pltpu.VMEM((D // 2, D), U32),
            pltpu.VMEM((NT_, 3 * D, 128), F32),
            pltpu.VMEM((3 * NT_, RB, 128), F32),
            pltpu.VMEM((3 * NT_, HALO + RB, 128), F32),
            pltpu.VMEM((RB, D), F32),
            pltpu.VMEM((RB, D), F32),
            pltpu.VMEM((2, RB // 2, D), U32),
            pltpu.SemaphoreType.DMA((NP,)),
            pltpu.SemaphoreType.DMA((11,)),
            pltpu.SemaphoreType.DMA((1,)),
        ],
        compiler_params=pltpu.CompilerParams(vmem_limit_bytes=120 * 1024 * 1024,
                                             disable_bounds_checks=True),
    )(A_x.reshape(S, D), A_mem0.reshape(M, D), wt(A_Wq), wt(A_Wk), wt(A_Wv),
      A_Wo.reshape(H * DH, D), B_wqkv, B_wo, gate_w)
    return out.reshape(1, S, D)
```

```python
import functools

import jax
import jax.numpy as jnp
from jax.experimental import pallas as pl
from jax.experimental.pallas import tpu as pltpu

F32 = jnp.float32
BF16 = jnp.bfloat16
U32 = jnp.uint32

S = 2048
D = 640
NT_ = D // 128
MASK_VALUE = -1e9
LOG2E = 1.4426950408889634
H = 32
DH = 192
M = 8
SEG = 32
L = M + SEG
NSEG = S // SEG
NP = H // 2
PW = 2 * DH
LAG_S, LAG_V, LAG_O = 1, 4, 8
SEG_UNROLL = 3
HB = 32
DB = D // HB
WIN = 8
DIL = 2
RB = 128
NB = S // RB
SUB = 64
HALO = 16
XA0 = 256
XA1 = 768
EARLY_PAIRS = 4
WO_SPLIT = 10

NN = (((1,), (0,)), ((), ()))
NT = (((1,), (1,)), ((), ()))


def _dot(a, b, dims=NN):
    return jax.lax.dot_general(a, b, dims, preferred_element_type=F32)


def _w(x):
    return pltpu.bitcast(x, BF16)


def _pack(x):
    return pltpu.bitcast(x, U32)


def _recip(den):
    r = pl.reciprocal(den, approx=True)
    return r * (2.0 - den * r)


def _blockdiag(t):
    lo = jax.lax.broadcasted_iota(jnp.int32, (L, 128), 1) < 64
    z = jnp.zeros((L, 128), F32)
    t0, t1, t2 = t[:, 0:128], t[:, 128:256], t[:, 256:384]
    top = jnp.concatenate([t0, jnp.where(lo, t1, 0.0), z], axis=1)
    bot = jnp.concatenate([z, jnp.where(lo, 0.0, t1), t2], axis=1)
    return jnp.concatenate([top, bot], axis=0).astype(BF16)


def _kernel(x_hbm, mem_hbm, wq_hbm, wk_hbm, wv_hbm, wo_hbm, wqkvb_hbm, wob_hbm, gate_hbm,
            out_hbm,
            x_v, out_v, b_v, h_ref, mem_v, gate_v,
            qkv_stage, wo_stage, w32, wo32,
            wqkvb_v, wob_v, wqkvb32, wob32, prep, fresh, cur, onew, ocur, x32,
            sem_qkv, sem_in, sem_out):
    def qkv_copies(p):
        rows = pl.ds(pl.multiple_of(p * PW, 128), PW)
        return [pltpu.make_async_copy(src.at[rows, :], qkv_stage.at[i, rows, :], sem_qkv.at[p])
                for i, src in enumerate((wq_hbm, wk_hbm, wv_hbm))]

    def start_qkv(pairs):
        for p in pairs:
            for c in qkv_copies(p):
                c.start(priority=1)

    def wait_qkv(p):
        for c in qkv_copies(p):
            c.wait()

    c_wqkvb = [pltpu.make_async_copy(wqkvb_hbm.at[:, i * D:(i + 1) * D],
                                     wqkvb_v.at[:, i * D:(i + 1) * D], sem_in.at[i])
               for i in range(3)]
    c_x = [pltpu.make_async_copy(x_hbm.at[lo:hi, :], x_v.at[lo:hi, :], sem_in.at[3 + i])
           for i, (lo, hi) in enumerate(((0, XA0), (XA0, XA1), (XA1, S)))]
    c_wob = pltpu.make_async_copy(wob_hbm, wob_v, sem_in.at[6])
    c_wo = [pltpu.make_async_copy(wo_hbm.at[lo * PW:hi * PW, :], wo_stage.at[lo * PW:hi * PW, :],
                                  sem_in.at[sem])
            for lo, hi, sem in ((0, WO_SPLIT, 7), (WO_SPLIT, NP, 10))]
    c_mem = pltpu.make_async_copy(mem_hbm, mem_v, sem_in.at[8])
    c_gate = pltpu.make_async_copy(gate_hbm, gate_v, sem_in.at[9])
    c_x[0].start()
    for c in c_wqkvb:
        c.start()
    for c in (c_wob, c_x[1], c_mem, c_gate):
        c.start(priority=1)

    def prep_wqkvb(part):
        for c in range(part * NT_, (part + 1) * NT_):
            t = wqkvb_v[:, c * 128:(c + 1) * 128].astype(F32).T
            for kt in range(NT_):
                prep[kt, c * 128:(c + 1) * 128, :] = t[:, kt * 128:(kt + 1) * 128]
        for d in range(DB):
            rows = jnp.concatenate(
                [prep[kt, pl.ds(part * D + d, HB, stride=DB), :] for kt in range(NT_)], axis=1)
            r0 = (part * D + d * HB) // 2
            wqkvb32[r0:r0 + HB // 2, :] = _pack(rows.astype(BF16))

    def prep_wob():
        for kt in range(NT_):
            prep[kt, 0:D, :] = wob_v[:, kt * 128:(kt + 1) * 128].astype(F32)
        for d in range(DB):
            rows = jnp.concatenate(
                [prep[kt, pl.ds(d, HB, stride=DB), :] for kt in range(NT_)], axis=1)
            wob32[d * (HB // 2):(d + 1) * (HB // 2), :] = _pack(rows.astype(BF16))

    def b_project(blk, part=None):
        xp = x32.at[0 if part is None else 1]
        if not part:
            xp[...] = _pack(x_v[pl.ds(pl.multiple_of(blk * RB, RB), RB), :])
        tiles = range(3 * NT_) if part is None else range(part * NT_, (part + 1) * NT_)
        for j in tiles:
            y = _dot(_w(xp[...]), _w(wqkvb32[j * 64:(j + 1) * 64, :]), NT)
            if part is None:
                fresh[j] = y
            else:
                cur[j, HALO:HALO + RB, :] = y
                if j >= NT_:
                    cur[j, 0:HALO, :] = jnp.zeros((HALO, 128), F32)

    def b_rotate():
        for j in range(NT_, 3 * NT_):
            cur[j, 0:HALO, :] = cur[j, RB:RB + HALO, :]
        for j in range(3 * NT_):
            cur[j, HALO:HALO + RB, :] = fresh[j]
        ocur[...] = onew[...]

    def b_attend_rows(base, n, first):
        q = [cur[j, HALO + base:HALO + base + n, :] for j in range(NT_)]
        row = jax.lax.broadcasted_iota(jnp.int32, (n, 128), 0) + base
        half = WIN // 2
        step = DIL * half
        logits = [None] * WIN
        for w in range(half):
            o = HALO + base - DIL * w - step
            lo = hi = None
            for j in range(NT_):
                k = cur[NT_ + j, o:o + n + step, :]
                a, b = q[j] * k[step:], q[j] * k[:n]
                lo = a if lo is None else lo + a
                hi = b if hi is None else hi + b
            for ww, s in ((w, lo), (w + half, hi)):
                s = s + pltpu.roll(s, 64, 1)
                s = s + pltpu.roll(s, 32, 1)
                s = s * (DB ** -0.5 * LOG2E)
                if first and base < DIL * ww:
                    s = jnp.where(row >= DIL * ww, s, MASK_VALUE * LOG2E)
                logits[ww] = s
        m = logits[0]
        for w in range(1, WIN):
            m = jnp.maximum(m, logits[w])
        e = [jnp.exp2(l - m) for l in logits]
        den = e[0]
        for w in range(1, WIN):
            den = den + e[w]
        r = _recip(den)
        outs = []
        for j in range(NT_):
            acc = None
            for w in range(half):
                o = HALO + base - DIL * w - step
                v = cur[2 * NT_ + j, o:o + n + step, :]
                t = e[w] * v[step:] + e[w + half] * v[:n]
                acc = t if acc is None else acc + t
            outs.append(acc * r)
        return jnp.concatenate(outs, axis=1)

    def b_attend(first=False):
        for base in range(0, RB, SUB):
            onew[base:base + SUB, :] = b_attend_rows(base, SUB, first)

    def b_output(blk, src):
        b_v[pl.ds(pl.multiple_of(blk * RB, RB), RB), :] = _dot(src[...], _w(wob32[...]))

    def a_qkv_weights(p):
        rows = pl.ds(pl.multiple_of(p * PW, 128), PW)
        col = pl.multiple_of(p * 3 * PW, 128)
        for i in range(3):
            w32[:, pl.ds(col + i * PW, PW)] = _pack(
                qkv_stage[i, rows, :].astype(F32).T.astype(BF16))

    c_x[0].wait()
    c_wqkvb[0].wait()
    start_qkv(range(EARLY_PAIRS))
    prep_wqkvb(0)
    c_wqkvb[1].wait()
    c_x[2].start(priority=1)
    prep_wqkvb(1)
    b_project(0, part=0)
    c_wqkvb[2].wait()
    start_qkv(range(EARLY_PAIRS, NP))
    prep_wqkvb(2)
    b_project(0, part=1)
    c_wob.wait()
    b_project(0, part=2)
    for c in c_wo:
        c.start(priority=1)
    b_project(1)
    b_attend(first=True)
    prep_wob()
    b_rotate()
    c_x[1].wait()
    c_mem.wait()
    c_gate.wait()

    def b_step(k, carry):
        @pl.when(k == XA1 // RB - 1)
        def _():
            c_x[2].wait()

        wait_qkv(k - 1)
        b_project(k + 1)
        b_output(k - 1, ocur)
        b_attend()
        a_qkv_weights(k - 1)
        b_rotate()
        return carry

    jax.lax.fori_loop(1, NB - 1, b_step, 0)

    h_ref[SEG:L, :] = mem_v[...].astype(F32)
    gate = gate_v[...].astype(F32).reshape(1, D)

    def segment(s, first=False):
        off = s * SEG if first else pl.multiple_of(s * SEG, SEG)
        x = x_v[pl.ds(off, SEG), :].astype(F32)
        h_ref[0:SEG, :] = x
        r = jax.lax.broadcasted_iota(jnp.int32, (L, 2 * L), 0)
        c = jax.lax.broadcasted_iota(jnp.int32, (L, 2 * L), 1)
        isb = c >= L
        key = jnp.where(isb, c - L, c)
        allowed = (r >= SEG) | (key >= SEG) | (r >= key)
        st = [dict() for _ in range(NP)]
        acc = [None]

        def project(p):
            h = h_ref[...]
            b = p * 3 * PW
            if p == 0 and not first:
                q = None
                for kt in range(NT_):
                    t = _dot(h[:, kt * 128:(kt + 1) * 128],
                             _w(w32[kt * 64:(kt + 1) * 64, b:b + PW]))
                    q = t if q is None else q + t
            else:
                q = _dot(h, _w(w32[:, b:b + PW]))
            st[p]['q'] = q
            st[p]['kb'] = _blockdiag(_dot(h, _w(w32[:, b + PW:b + 2 * PW])))
            st[p]['vb'] = _blockdiag(_dot(h, _w(w32[:, b + 2 * PW:b + 3 * PW])))

        def softmax(p):
            sc = _dot(st[p].pop('q'), st[p].pop('kb'), NT)
            t = jnp.where(allowed, sc * (DH ** -0.5 * LOG2E), MASK_VALUE * LOG2E)
            ma = jnp.max(jnp.where(isb, -jnp.inf, t), axis=1, keepdims=True)
            mb = jnp.max(jnp.where(isb, t, -jnp.inf), axis=1, keepdims=True)
            e = jnp.exp2(t - jnp.where(isb, mb, ma))
            sa = jnp.sum(jnp.where(isb, 0.0, e), axis=1, keepdims=True)
            sb = jnp.sum(jnp.where(isb, e, 0.0), axis=1, keepdims=True)
            st[p]['p'] = e * _recip(jnp.where(isb, sb, sa))

        def values(p):
            st[p]['o'] = _dot(st[p].pop('p'), st[p].pop('vb'))

        def output(p):
            if first:
                w = wo_stage[p * PW:(p + 1) * PW, :]
                wo32[p * (PW // 2):(p + 1) * (PW // 2), :] = _pack(w)
            else:
                w = _w(wo32[p * (PW // 2):(p + 1) * (PW // 2), :])
            o = st[p].pop('o')
            y = _dot(jnp.concatenate([o[SEG:L], o[0:SEG]], axis=0), w)
            acc[0] = y if acc[0] is None else acc[0] + y

        for t in range(NP + (LAG_V + 1 if first else LAG_O)):
            if t < NP:
                project(t)
            if first and t == 0:
                b_attend()
            if first and t == NP:
                b_output(NB - 1, onew)
            if 0 <= t - LAG_S < NP:
                softmax(t - LAG_S)
            if 0 <= t - LAG_V < NP:
                values(t - LAG_V)
            if not first and 0 <= t - LAG_O < NP:
                output(t - LAG_O)
            if first and t >= NP + 2:
                if t == NP + 2:
                    c_wo[0].wait()
                j = t - (NP + 2)
                for p in range(4 * j, min(4 * j + 4, WO_SPLIT)):
                    output(p)
        if first:
            c_wo[1].wait()
            for p in range(WO_SPLIT, NP):
                output(p)
        a = acc[0]
        h_ref[SEG:L, :] = a[0:M]
        z = jnp.sum(x * gate, axis=1, keepdims=True)
        g = 1.0 / (1.0 + jnp.exp(-z))
        y = g * a[M:L] + (1.0 - g) * b_v[pl.ds(off, SEG), :]
        out_v[pl.ds(off, SEG), :] = y.astype(out_v.dtype)
        pltpu.make_async_copy(out_v.at[pl.ds(off, SEG), :], out_hbm.at[pl.ds(off, SEG), :],
                              sem_out.at[0]).start()

    def first_segment(i, carry):
        wait_qkv(NB - 2)
        wait_qkv(NB - 1)
        b_output(NB - 2, ocur)
        a_qkv_weights(NB - 2)
        a_qkv_weights(NB - 1)
        segment(0, first=True)
        return carry

    jax.lax.fori_loop(0, pl.program_id(0) + 1, first_segment, 0)

    def segments(i, carry):
        for u in range(SEG_UNROLL):
            segment(1 + i * SEG_UNROLL + u)
        return carry

    jax.lax.fori_loop(0, (NSEG - 1) // SEG_UNROLL, segments, 0)
    pltpu.make_async_copy(out_v, out_hbm, sem_out.at[0]).wait()


@functools.partial(jax.jit, static_argnames=("A_seg_len",))
def pallas_gated_mix__memory_aug_recurrent_mem_tr__sliding_local_dilated__prompt_kernel(
    A_x: jax.Array,
    A_mem0: jax.Array,
    A_Wq: jax.Array,
    A_Wk: jax.Array,
    A_Wv: jax.Array,
    A_Wo: jax.Array,
    A_seg_len: int,
    B_x: jax.Array,
    B_wqkv: jax.Array,
    B_wo: jax.Array,
    gate_w: jax.Array,
):
    del B_x
    assert A_seg_len == SEG and (NSEG - 1) % SEG_UNROLL == 0
    assert A_x.shape == (1, S, D) and A_Wq.shape == (D, H, DH) and A_mem0.shape == (1, M, D)

    def wt(w):
        return jnp.transpose(w, (1, 2, 0)).reshape(H * DH, D)

    hbm = pl.BlockSpec(memory_space=pl.ANY)
    out = pl.pallas_call(
        _kernel,
        out_shape=jax.ShapeDtypeStruct((S, D), BF16),
        in_specs=[hbm] * 9,
        out_specs=hbm,
        grid=(1,),
        scratch_shapes=[
            pltpu.VMEM((S, D), BF16),
            pltpu.VMEM((S, D), BF16),
            pltpu.VMEM((S, D), F32),
            pltpu.VMEM((L, D), F32),
            pltpu.VMEM((M, D), BF16),
            pltpu.VMEM((D,), BF16),
            pltpu.VMEM((3, H * DH, D), BF16),
            pltpu.VMEM((H * DH, D), BF16),
            pltpu.VMEM((D // 2, 3 * H * DH), U32),
            pltpu.VMEM((H * DH // 2, D), U32),
            pltpu.VMEM((D, 3 * D), BF16),
            pltpu.VMEM((D, D), BF16),
            pltpu.VMEM((3 * D // 2, D), U32),
            pltpu.VMEM((D // 2, D), U32),
            pltpu.VMEM((NT_, 3 * D + HB, 128), F32),
            pltpu.VMEM((3 * NT_, RB, 128), F32),
            pltpu.VMEM((3 * NT_, HALO + RB, 128), F32),
            pltpu.VMEM((RB, D), F32),
            pltpu.VMEM((RB, D), F32),
            pltpu.VMEM((2, RB // 2, D), U32),
            pltpu.SemaphoreType.DMA((NP,)),
            pltpu.SemaphoreType.DMA((11,)),
            pltpu.SemaphoreType.DMA((1,)),
        ],
        compiler_params=pltpu.CompilerParams(vmem_limit_bytes=120 * 1024 * 1024,
                                             disable_bounds_checks=True),
    )(A_x.reshape(S, D), A_mem0.reshape(M, D), wt(A_Wq), wt(A_Wk), wt(A_Wv),
      A_Wo.reshape(H * DH, D), B_wqkv, B_wo, gate_w)
    return out.reshape(1, S, D)
```
